```python
import jax
import jax.numpy as jnp

def _softmax(x, axis=-1):
    return jax.nn.softmax(x, axis=axis)
def _gelu(x):
    return jax.nn.gelu(x, approximate=True)
def _silu(x):
    return jax.nn.silu(x)
def _sigmoid(x):
    return jax.nn.sigmoid(x)
def _layernorm(x, axis=-1, eps=1e-5):
    m = jnp.mean(x, axis=axis, keepdims=True)
    v = jnp.var(x, axis=axis, keepdims=True)
    return (x - m) / jnp.sqrt(v + eps)
def _scatter_add(tgt, idx, src, axis=0):
    return tgt.at[idx].add(src)
def _segment_sum(src, seg, n):
    return jax.ops.segment_sum(src, seg, n)
class _Rng:
    def __init__(self, key):
        self._k = key
    def _next(self):
        self._k, sub = jax.random.split(self._k)
        return sub
    def normal(self, shape):
        return jax.random.normal(self._next(), shape, dtype=jnp.bfloat16)
    def randint(self, lo, hi, shape):
        return jax.random.randint(self._next(), shape, lo, hi, dtype=jnp.int32)
    def uniform(self, shape, lo=0.0, hi=1.0):
        return jax.random.uniform(self._next(), shape, jnp.bfloat16, lo, hi)
    def permutation(self, n):
        return jax.random.permutation(self._next(), n)


kernel_name = 'standalone__seq2seq_rnn_t_joint__speech'

def setup_inputs():
    _rng = _Rng(jax.random.key(int.from_bytes(__import__("os").urandom(4), "little")))
    _w = (lambda a: (lambda t: t.astype(jnp.bfloat16) if jnp.issubdtype(t.dtype, jnp.floating) else t)(jnp.asarray(a)))
    B, T, D, K = 2, 16000, 256, 31
    U = 8
    sc = (1.0 / (K * D)) ** 0.5
    sd = (1.0 / D) ** 0.5
    return {
        "x": _w((lambda *s: _rng.normal(s) * 0.05)(B, T, D) * 0.5),
        "w1": _w((lambda *s: _rng.normal(s) * 0.05)(K, D, D) * sc),
        "w2": _w((lambda *s: _rng.normal(s) * 0.05)(K, D, D) * sc),
        "g": _w((lambda *s: _rng.normal(s) * 0.05)(B, U, D) * 0.5),
        "w_f": _w((lambda *s: _rng.normal(s) * 0.05)(D, D) * sd),
        "w_g": _w((lambda *s: _rng.normal(s) * 0.05)(D, D) * sd),
        "w_o": _w((lambda *s: _rng.normal(s) * 0.05)(D, D) * sd),
    }

def reference(x, w1, w2, g, w_f, w_g, w_o):
    B, T, D = x.shape
    K = w1.shape[0]
    pad = K // 2
    xp = jnp.pad(x, ((0,0),(pad,pad),(0,0)))
    h = jnp.zeros_like(x)
    for i in range(K):
        h = h + jnp.einsum("btc,cd->btd", xp[:, i:i+T, :], w1[i])
    h = _gelu(h)[:, ::2, :]
    T1 = h.shape[1]
    hp = jnp.pad(h, ((0,0),(pad,pad),(0,0)))
    f = jnp.zeros_like(h)
    for i in range(K):
        f = f + jnp.einsum("btc,cd->btd", hp[:, i:i+T1, :], w2[i])
    f = _gelu(f)[:, ::2, :]
    fe = jnp.einsum("btd,de->bte", f, w_f)
    ge = jnp.einsum("bud,de->bue", g, w_g)
    j = jnp.tanh(fe[:, :, None, :] + ge[:, None, :, :])
    return jnp.einsum("btud,dv->btuv", j, w_o)
```

```python
import functools, math
import jax
import jax.numpy as jnp
import numpy as np
from jax import lax
from jax.experimental import pallas as pl
from jax.experimental.pallas import tpu as pltpu

F32, BF16, U32 = jnp.float32, jnp.bfloat16, jnp.uint32
R = 128
JT = 125
XPAD = 33
GP = 8


def _bc(x, ty):
    return pltpu.bitcast(x, ty)


def _expand(a):
    if len(a) == 1:
        return [a[0]]
    m = len(a) // 2
    lo, hi = a[:m], a[m:]
    return _expand(lo) + _expand(hi) + _expand([p - q for p, q in zip(lo, hi)])


def _comb(p0, p1, p2, m):
    n = 2 * m - 1
    mid = [p0[k] + p1[k] - p2[k] for k in range(n)]
    out = []
    for k in range(4 * m - 1):
        terms = []
        if k < n:
            terms.append(p0[k])
        if 0 <= k - m < n:
            terms.append(mid[k - m])
        if 0 <= k - 2 * m < n:
            terms.append(p1[k - 2 * m])
        s = terms[0]
        for t in terms[1:]:
            s = s + t
        out.append(s)
    return out


def _interp(p):
    if len(p) == 1:
        return [p[0]]
    n3 = len(p) // 3
    L = round(math.log(len(p), 3))
    ch = [_interp(p[i * n3:(i + 1) * n3]) for i in range(3)]
    return _comb(ch[0], ch[1], ch[2], 2 ** (L - 1))


def _gelu(y):
    c = 0.7978845608028654
    inner = y * (c + (c * 0.044715) * (y * y))
    return (0.5 * y) * (1.0 + jnp.tanh(inner))


def kernel(x_hbm, w1_hbm, w2_hbm, g_ref, wf_ref, wg_ref, wo_ref, o_ref,
           xbuf, xs, wst, wt1, wt2, lsc, psc, gsc, hsc, fsc, fesc, gesc, wfs, wos, sem):
    tile = pl.program_id(0)
    half = tile % 2
    b = tile // 2

    def x_copy(t):
        bb = t // 2
        hf = t % 2
        c0 = pltpu.make_async_copy(x_hbm.at[bb, pl.ds(0, 8128)], xbuf.at[0, pl.ds(64, 8128)], sem.at[0])
        c1 = pltpu.make_async_copy(x_hbm.at[bb, pl.ds(7936, 8064)], xbuf.at[1, pl.ds(0, 8064)], sem.at[1])
        return hf, c0, c1

    def x_start(t):
        hf, c0, c1 = x_copy(t)
        pl.when(hf == 0)(c0.start)
        pl.when(hf == 1)(c1.start)

    def x_wait(t):
        hf, c0, c1 = x_copy(t)
        pl.when(hf == 0)(c0.wait)
        pl.when(hf == 1)(c1.wait)

    def transform_w(w_hbm, wt):
        cp = pltpu.make_async_copy(w_hbm, wst, sem.at[2])
        cp.start()
        cp.wait()

        def body(i, carry):
            r0 = pl.multiple_of(i * 32, 32)
            for e in range(2):
                for ct in range(2):
                    taps = []
                    for j in range(16):
                        idx = 29 - 2 * j + e
                        if idx < 0:
                            taps.append(jnp.zeros((32, 128), F32))
                        else:
                            taps.append(wst[idx, pl.ds(r0, 32), pl.ds(128 * ct, 128)].astype(F32))
                    lv = _expand(taps)
                    for q in range(81):
                        wt[q, pl.ds(pl.multiple_of(128 * e + i * 16, 16), 16), pl.ds(128 * ct, 128)] = _bc(lv[q].astype(BF16), U32)
            return carry
        lax.fori_loop(0, 8, body, 0)

    @pl.when(tile == 0)
    def _():
        x_start(tile)
        xbuf[0, pl.ds(0, 64), :] = jnp.zeros((64, 256), BF16)
        xbuf[1, pl.ds(8064, 128), :] = jnp.zeros((128, 256), BF16)
        gsc[...] = jnp.zeros(gsc.shape, F32)
        wfs[...] = _bc(wf_ref[...], U32)
        wos[...] = _bc(wo_ref[...], U32)
        for bb in range(2):
            gesc[bb] = jnp.dot(g_ref[bb], wg_ref[...], preferred_element_type=F32)
        transform_w(w1_hbm, wt1)
        transform_w(w2_hbm, wt2)

    x_wait(tile)

    @pl.when(tile + 1 < pl.num_programs(0))
    def _():
        x_start(tile + 1)

    for rho in range(R):
        slot = 32 * (rho % 4) + rho // 4
        for ct in range(2):
            xs[ct, pl.ds(XPAD * slot, 32), :] = _bc(xbuf[half, pl.ds(64 * rho, 64), pl.ds(128 * ct, 128)], U32)

    def raw_x(c):
        def load(r, kap, q, ab):
            e, ct = divmod(kap, 2)
            cls = (q // 4) + 2 * ab
            w = xs[ct, pl.ds(XPAD * (32 * cls + 8 * (q % 4)) + 16 * c + r, 8, stride=XPAD), :]
            if e == 0:
                return _bc(w << 16, F32)
            return _bc(w & np.uint32(0xFFFF0000), F32)
        return load

    def raw_h(r, kap, q, ab):
        e, ct = divmod(kap, 2)
        return hsc[2 * r + e, ct, pl.ds(64 * ab + 8 * q, 8), :]

    def pre_item(load, g, slot, q, kap):
        lv = []
        for ab in range(2):
            if g == 0:
                a = [load(r, kap, q, ab) for r in range(8)]
            elif g == 1:
                a = [load(r + 8, kap, q, ab) for r in range(8)]
            else:
                a = [load(r, kap, q, ab) - load(r + 8, kap, q, ab) for r in range(8)]
            lv.append(_expand(a))
        for l in range(27):
            lsc[slot, l, pl.ds(8 * q, 8), pl.ds(128 * kap, 128)] = pltpu.pack_elementwise(
                [lv[0][l], lv[1][l]], packed_dtype=BF16)

    def mm_item(wt, g, slot, q):
        lhs = _bc(lsc[slot, q], BF16)
        rhs = _bc(wt[27 * g + q], BF16)
        res = jnp.dot(lhs, rhs, preferred_element_type=F32)
        for ct in range(2):
            psc[slot, q, ct] = res[:, 128 * ct:128 * (ct + 1)]

    def post_item(gslot, g, slot, chunk, ct):
        row0 = 16 * chunk
        p = [psc[slot, q, ct, pl.ds(row0, 16), :] for q in range(27)]
        co = _interp(p)
        for k in range(15):
            gsc[gslot, g, k, ct, pl.ds(GP + row0, 16), :] = co[k]

    def G(gslot, g, k, ct, row, n):
        return gsc[gslot, g, k, ct, pl.ds(GP + row, n), :]

    def own(gslot, r, ct, row, n):
        def M(k):
            return G(gslot, 0, k, ct, row, n) + G(gslot, 1, k, ct, row, n) - G(gslot, 2, k, ct, row, n)
        if r == 0:
            return G(gslot, 0, 7, ct, row, n)
        if r <= 7:
            return G(gslot, 0, r + 7, ct, row, n) + M(r - 1)
        if r == 8:
            return M(7)
        return G(gslot, 1, r - 9, ct, row, n) + M(r - 1)

    def final1_item(q, eo, ct):
        row = 64 * eo + 8 * q
        need_mask = eo == 0 and q in (0, 7)
        if need_mask:
            rows = lax.broadcasted_iota(jnp.int32, (8, 128), 0)
            bad = jnp.where(half == 0, 0, 8) if q == 0 else jnp.where(half == 0, 8, 7)
            keep = rows != bad
        prev_row = (64 + 8 * q - 1) if eo == 0 else 8 * q
        next_row = (64 + 8 * q) if eo == 0 else 8 * q + 1
        for c in range(2):
            for r in range(16):
                y = own(c, r, ct, row, 8)
                if r <= 7:
                    y = y + (G(1, 1, r + 7, ct, prev_row, 8) if c == 0 else G(0, 1, r + 7, ct, row, 8))
                if r >= 9:
                    y = y + (G(1, 0, r - 9, ct, row, 8) if c == 0 else G(0, 0, r - 9, ct, next_row, 8))
                h = _gelu(y)
                if need_mask:
                    h = jnp.where(keep, h, 0.0)
                hsc[16 * c + r, ct, pl.ds(row, 8), :] = h

    def final2_item(chunk, ct):
        row0 = 16 * chunk
        for r in range(16):
            y = own(2, r, ct, row0, 16)
            if r <= 7:
                y = y + G(2, 1, r + 7, ct, row0 - 1, 16)
            if r >= 9:
                y = y + G(2, 0, r - 9, ct, row0 + 1, 16)
            f = _gelu(y)
            fsc[r, pl.ds(8 * chunk, 8), pl.ds(128 * ct, 128)] = pltpu.pack_elementwise(
                [f[0:8], f[8:16]], packed_dtype=BF16)

    def conv_unit(load, wt, gslot):
        for g in range(3):
            for q in range(8):
                for kap in range(4):
                    pre_item(load, g, g % 2, q, kap)
            for q in range(27):
                mm_item(wt, g, g % 2, q)
            for chunk in range(8):
                for ct in range(2):
                    post_item(gslot, g, g % 2, chunk, ct)

    conv_unit(raw_x(0), wt1, 0)
    conv_unit(raw_x(1), wt1, 1)
    for q in range(8):
        for eo in range(2):
            for ct in range(2):
                final1_item(q, eo, ct)
    conv_unit(raw_h, wt2, 2)
    for chunk in range(8):
        for ct in range(2):
            final2_item(chunk, ct)

    wf = _bc(wfs[...], BF16)
    for r in range(16):
        fesc[r] = jnp.dot(_bc(fsc[r], BF16), wf, preferred_element_type=F32)

    ge = gesc[b]
    wo = _bc(wos[...], BF16)
    for i in range(JT):
        rho = i + 1
        m = 16 * (rho // 16) + (2 * (rho % 16) if rho % 16 < 8 else 2 * (rho % 16 - 8) + 1)
        rows = [jnp.tanh(fesc[r, pl.ds(m, 1), :] + ge) for r in range(16)]
        j = jnp.concatenate(rows, axis=0).astype(BF16)
        res = jnp.dot(j, wo, preferred_element_type=F32)
        o_ref[pl.ds(16 * i, 16)] = res.reshape(16, 8, 256).astype(BF16)


@jax.jit
def pallas_standalone__seq2seq_rnn_t_joint__speech_kernel(x, w1, w2, g, w_f, w_g, w_o):
    B, T, D = x.shape
    U = g.shape[1]
    assert (B, T, D, U) == (2, 16000, 256, 8) and w1.shape == (31, 256, 256)
    full = lambda shp: pl.BlockSpec(shp, lambda i: (0,) * len(shp))
    return pl.pallas_call(
        kernel,
        out_shape=jax.ShapeDtypeStruct((B, T // 4, U, D), x.dtype),
        grid=(4,),
        in_specs=[pl.BlockSpec(memory_space=pl.ANY)] * 3 + [full((B, U, D)), full((D, D)), full((D, D)), full((D, D))],
        out_specs=pl.BlockSpec((None, 2000, U, D), lambda i: (i // 2, i % 2, 0, 0)),
        scratch_shapes=[
            pltpu.VMEM((2, 8192, 256), BF16),
            pltpu.VMEM((2, XPAD * R, 128), U32),
            pltpu.VMEM((31, 256, 256), BF16),
            pltpu.VMEM((81, 256, 256), U32),
            pltpu.VMEM((81, 256, 256), U32),
            pltpu.VMEM((2, 27, 64, 512), U32),
            pltpu.VMEM((2, 27, 2, 128, 128), F32),
            pltpu.VMEM((3, 3, 15, 2, 144, 128), F32),
            pltpu.VMEM((32, 2, 128, 128), F32),
            pltpu.VMEM((16, 64, 256), U32),
            pltpu.VMEM((16, 128, 256), F32),
            pltpu.VMEM((2, 8, 256), F32),
            pltpu.VMEM((128, 256), U32),
            pltpu.VMEM((128, 256), U32),
            pltpu.SemaphoreType.DMA((3,)),
        ],
        compiler_params=pltpu.CompilerParams(
            dimension_semantics=("arbitrary",),
            vmem_limit_bytes=127 * 1024 * 1024,
        ),
    )(x, w1, w2, g, w_f, w_g, w_o)
```

```python
import functools, math
import jax
import jax.numpy as jnp
import numpy as np
from jax import lax
from jax.experimental import pallas as pl
from jax.experimental.pallas import tpu as pltpu

F32, BF16, U32 = jnp.float32, jnp.bfloat16, jnp.uint32
R = 128
JT = 125
XPAD = 33
GP = 8
NCH = 5
CH = JT // NCH
NTILE = 4
HI_MASK = np.uint32(0xFFFF0000)


def _bc(x, ty):
    return pltpu.bitcast(x, ty)


def _pack(a, b):
    return pltpu.pack_elementwise([a, b], packed_dtype=BF16)


def _lo(w):
    return _bc(w << 16, F32)


def _hi(w):
    return _bc(w & HI_MASK, F32)


def _expand(a):
    if len(a) == 1:
        return [a[0]]
    m = len(a) // 2
    lo, hi = a[:m], a[m:]
    return _expand(lo) + _expand(hi) + _expand([p - q for p, q in zip(lo, hi)])


def _comb(p0, p1, p2, m):
    n = 2 * m - 1
    mid = [p0[k] + p1[k] - p2[k] for k in range(n)]
    out = []
    for k in range(4 * m - 1):
        terms = []
        if k < n:
            terms.append(p0[k])
        if 0 <= k - m < n:
            terms.append(mid[k - m])
        if 0 <= k - 2 * m < n:
            terms.append(p1[k - 2 * m])
        s = terms[0]
        for t in terms[1:]:
            s = s + t
        out.append(s)
    return out


def _interp(p):
    if len(p) == 1:
        return [p[0]]
    n3 = len(p) // 3
    L = round(math.log(len(p), 3))
    ch = [_interp(p[i * n3:(i + 1) * n3]) for i in range(3)]
    return _comb(ch[0], ch[1], ch[2], 2 ** (L - 1))


def _gelu(y):
    c = 0.7978845608028654
    inner = y * (c + (c * 0.044715) * (y * y))
    return (0.5 * y) * (1.0 + jnp.tanh(inner))


def _interleave(backbone, fillers):
    nb, nf = len(backbone), len(fillers)
    done = 0
    for i, bb in enumerate(backbone):
        bb()
        upto = ((i + 1) * nf) // nb
        while done < upto:
            fillers[done]()
            done += 1
    while done < nf:
        fillers[done]()
        done += 1


def kernel(x_hbm, w1_hbm, w2_hbm, g_ref, wf_ref, wg_ref, wo_ref, o_hbm,
           xbuf, xs, wst1, wst2, wts, raws, lsc, psc, gsc, fsc, fesc, gesc, wfs, wos, ost,
           xsem, wsem, osem):
    k = pl.program_id(0)
    tile = k // 3
    ph = k % 3

    def x_copy(t, hf):
        bb = t // 2
        if hf == 0:
            return pltpu.make_async_copy(x_hbm.at[bb, pl.ds(0, 8128)], xbuf.at[pl.ds(64, 8128)], xsem.at[0])
        return pltpu.make_async_copy(x_hbm.at[bb, pl.ds(7936, 8064)], xbuf.at[pl.ds(0, 8064)], xsem.at[0])

    def x_start(t):
        def act(hf):
            x_copy(t, hf).start()
            lo, n = (0, 64) if hf == 0 else (8064, 128)
            xbuf[pl.ds(lo, n), :] = jnp.zeros((n, 256), BF16)
        if isinstance(t, int):
            act(t % 2)
        else:
            pl.when(t % 2 == 0)(functools.partial(act, 0))
            pl.when(t % 2 == 1)(functools.partial(act, 1))

    def x_wait(t):
        def act(hf):
            x_copy(t, hf).wait()
        if isinstance(t, int):
            act(t % 2)
        else:
            pl.when(t % 2 == 0)(functools.partial(act, 0))
            pl.when(t % 2 == 1)(functools.partial(act, 1))

    def o_copy(t, c):
        return pltpu.make_async_copy(
            ost.at[c], o_hbm.at[t // 2, pl.ds((t % 2) * 2000 + c * CH * 16, CH * 16)], osem.at[c])

    def transform_w(wst, cv):
        def body(i, carry):
            r0 = pl.multiple_of(i * 16, 16)
            for e in range(2):
                for ct in range(2):
                    lo, hi = [], []
                    for j in range(16):
                        idx = 29 - 2 * j + e
                        if idx < 0:
                            lo.append(jnp.zeros((8, 128), F32))
                            hi.append(jnp.zeros((8, 128), F32))
                        else:
                            w = _bc(wst[idx, pl.ds(r0, 16), pl.ds(128 * ct, 128)], U32)
                            lo.append(_lo(w))
                            hi.append(_hi(w))
                    la, lb = _expand(lo), _expand(hi)
                    for q in range(81):
                        wts[cv, q, pl.ds(pl.multiple_of(128 * e + i * 8, 8), 8), pl.ds(128 * ct, 128)] = _pack(la[q], lb[q])
            return carry
        lax.fori_loop(0, 16, body, 0)

    def xcopy_item(rho, ct):
        def f():
            slot = 32 * (rho % 4) + rho // 4
            xs[ct, pl.ds(XPAD * slot, 32), :] = _bc(xbuf[pl.ds(64 * rho, 64), pl.ds(128 * ct, 128)], U32)
        return f

    def xcopy_items():
        return [xcopy_item(rho, ct) for rho in range(R) for ct in range(2)]

    def rawprep_item(c, r, ct):
        def f():
            for q in range(8):
                for ab in range(2):
                    cls = (q // 4) + 2 * ab
                    raws[c, r, ct, pl.ds(64 * ab + 8 * q, 8), :] = xs[
                        ct, pl.ds(XPAD * (32 * cls + 8 * (q % 4)) + 16 * c + r, 8, stride=XPAD), :]
        return f

    def rawprep_items():
        return [rawprep_item(c, r, ct) for c in range(2) for r in range(16) for ct in range(2)]

    def pre_item(rs, g, q, kap):
        def f():
            e, ct = divmod(kap, 2)
            un = _lo if e == 0 else _hi

            def load(r, ab):
                return un(raws[rs, r, ct, pl.ds(64 * ab + 8 * q, 8), :])
            lv = []
            for ab in range(2):
                if g == 0:
                    a = [load(r, ab) for r in range(8)]
                elif g == 1:
                    a = [load(r + 8, ab) for r in range(8)]
                else:
                    a = [load(r, ab) - load(r + 8, ab) for r in range(8)]
                lv.append(_expand(a))
            for l in range(27):
                lsc[g, l, pl.ds(8 * q, 8), pl.ds(128 * kap, 128)] = _pack(lv[0][l], lv[1][l])
        return f

    def pre_items(rs, g):
        return [pre_item(rs, g, q, kap) for q in range(8) for kap in range(4)]

    def mm_item(cv, g, l):
        def f():
            lhs = _bc(lsc[g, l], BF16)
            rhs = _bc(wts[cv, 27 * g + l], BF16)
            res = jnp.dot(lhs, rhs, preferred_element_type=F32)
            for ct in range(2):
                psc[g, l, ct] = res[:, 128 * ct:128 * (ct + 1)]
        return f

    def mm_items(cv, g):
        return [mm_item(cv, g, l) for l in range(27)]

    def post_item(gslot, g, chunk, ct):
        def f():
            row0 = 16 * chunk
            p = [psc[g, l, ct, pl.ds(row0, 16), :] for l in range(27)]
            co = _interp(p)
            for kk in range(15):
                gsc[gslot, g, kk, ct, pl.ds(GP + row0, 16), :] = co[kk]
        return f

    def post_items(gslot, g):
        return [post_item(gslot, g, chunk, ct) for chunk in range(8) for ct in range(2)]

    def G(gslot, g, kk, ct, row, n):
        return gsc[gslot, g, kk, ct, pl.ds(GP + row, n), :]

    def own(gslot, r, ct, row, n):
        def M(kk):
            return G(gslot, 0, kk, ct, row, n) + G(gslot, 1, kk, ct, row, n) - G(gslot, 2, kk, ct, row, n)
        if r == 0:
            return G(gslot, 0, 7, ct, row, n)
        if r <= 7:
            return G(gslot, 0, r + 7, ct, row, n) + M(r - 1)
        if r == 8:
            return M(7)
        return G(gslot, 1, r - 9, ct, row, n) + M(r - 1)

    def final1_item(t, q, eo, ct):
        def f():
            half = t % 2
            row = 64 * eo + 8 * q
            need_mask = eo == 0 and q in (0, 7)
            if need_mask:
                rows = lax.broadcasted_iota(jnp.int32, (8, 128), 0)
                bad = jnp.where(half == 0, 0, 8) if q == 0 else jnp.where(half == 0, 8, 7)
                keep = rows != bad
            prev_row = (64 + 8 * q - 1) if eo == 0 else 8 * q
            next_row = (64 + 8 * q) if eo == 0 else 8 * q + 1
            for c in range(2):
                hs = []
                for r in range(16):
                    y = own(c, r, ct, row, 8)
                    if r <= 7:
                        y = y + (G(1, 1, r + 7, ct, prev_row, 8) if c == 0 else G(0, 1, r + 7, ct, row, 8))
                    if r >= 9:
                        y = y + (G(1, 0, r - 9, ct, row, 8) if c == 0 else G(0, 0, r - 9, ct, next_row, 8))
                    h = _gelu(y)
                    if need_mask:
                        h = jnp.where(keep, h, 0.0)
                    hs.append(h)
                for rp in range(8):
                    raws[2, 8 * c + rp, ct, pl.ds(row, 8), :] = _pack(hs[2 * rp], hs[2 * rp + 1])
        return f

    def final1_items(t):
        return [final1_item(t, q, eo, ct) for q in range(8) for eo in range(2) for ct in range(2)]

    def final2_item(chunk, ct):
        def f():
            row0 = 16 * chunk
            for r in range(16):
                y = own(2, r, ct, row0, 16)
                if r <= 7:
                    y = y + G(2, 1, r + 7, ct, row0 - 1, 16)
                if r >= 9:
                    y = y + G(2, 0, r - 9, ct, row0 + 1, 16)
                fv = _gelu(y)
                fsc[r, pl.ds(8 * chunk, 8), pl.ds(128 * ct, 128)] = _pack(fv[0:8], fv[8:16])
        return f

    def final2_items():
        return [final2_item(chunk, ct) for chunk in range(8) for ct in range(2)]

    def fe_item(r):
        def f():
            fesc[r] = jnp.dot(_bc(fsc[r], BF16), _bc(wfs[...], BF16), preferred_element_type=F32)
        return f

    def fe_items():
        return [fe_item(r) for r in range(16)]

    def joint_item(t, i):
        def f():
            rho = i + 1
            m = 16 * (rho // 16) + (2 * (rho % 16) if rho % 16 < 8 else 2 * (rho % 16 - 8) + 1)
            ge = gesc[t // 2]
            rows = [jnp.tanh(fesc[r, pl.ds(m, 1), :] + ge) for r in range(16)]
            j = jnp.concatenate(rows, axis=0).astype(BF16)
            res = jnp.dot(j, _bc(wos[...], BF16), preferred_element_type=F32)
            c, ii = divmod(i, CH)
            ost[c, pl.ds(16 * ii, 16)] = res.reshape(16, 8, 256).astype(BF16)
            if ii == CH - 1:
                o_copy(t, c).start()
        return f

    def joint_items(t):
        return [joint_item(t, i) for i in range(JT)]

    def gap_items(t):
        return (post_items(1, 2) + final1_items(t) + xcopy_items() + rawprep_items() + pre_items(2, 0))

    def unit_body():
        cv = jnp.where(ph == 2, 1, 0)
        nxt = (ph + 1) % 3
        prv = (ph + 2) % 3
        _interleave(mm_items(cv, 0), post_items(prv, 2) + pre_items(ph, 1))
        _interleave(mm_items(cv, 1), post_items(ph, 0) + pre_items(ph, 2))
        _interleave(mm_items(cv, 2), post_items(ph, 1) + pre_items(nxt, 0))

    @pl.when(k == 0)
    def _():
        cw1 = pltpu.make_async_copy(w1_hbm, wst1, wsem.at[0])
        cw2 = pltpu.make_async_copy(w2_hbm, wst2, wsem.at[1])
        cw1.start()
        x_start(0)
        cw2.start()
        for kk in range(15):
            for gg in range(2):
                gsc[2, gg, kk] = jnp.zeros((2, R + 2 * GP, 128), F32)
        for l in range(27):
            psc[2, l] = jnp.zeros((2, R, 128), F32)
        wfs[...] = _bc(wf_ref[...], U32)
        wos[...] = _bc(wo_ref[...], U32)
        for bb in range(2):
            gesc[bb] = jnp.dot(g_ref[bb], wg_ref[...], preferred_element_type=F32)
        cw1.wait()
        transform_w(wst1, 0)
        x_wait(0)
        for it in xcopy_items() + rawprep_items() + pre_items(0, 0):
            it()
        cw2.wait()
        transform_w(wst2, 1)

    @pl.when(jnp.logical_and(ph == 0, tile + 1 < NTILE))
    def _():
        x_start(tile + 1)

    mid = jnp.logical_or(ph == 2, k == 3 * NTILE)

    @pl.when(jnp.logical_and(ph == 2, tile + 1 < NTILE))
    def _():
        x_wait(tile + 1)

    @pl.when(jnp.logical_and(mid, k > 5))
    def _():
        for c in range(NCH):
            o_copy(0, c).wait()

    @pl.when(k == 2)
    def _():
        with jax.named_scope('B0'):
            for it in gap_items(tile):
                it()

    @pl.when(k == 3 * NTILE)
    def _():
        with jax.named_scope('tail'):
            for it in post_items(2, 2):
                it()

    @pl.when(jnp.logical_and(mid, k > 2))
    def _():
        with jax.named_scope('B1'):
            jt = jnp.where(k == 3 * NTILE, NTILE - 1, tile - 1)
            for it in final2_items() + fe_items():
                it()
            _interleave(joint_items(jt), gap_items(tile))

    @pl.when(k < 3 * NTILE)
    def _():
        with jax.named_scope('unit'):
            unit_body()

    @pl.when(k == 3 * NTILE)
    def _():
        for c in range(NCH):
            o_copy(0, c).wait()


@jax.jit
def pallas_standalone__seq2seq_rnn_t_joint__speech_kernel(x, w1, w2, g, w_f, w_g, w_o):
    B, T, D = x.shape
    U = g.shape[1]
    assert (B, T, D, U) == (2, 16000, 256, 8) and w1.shape == (31, 256, 256)
    full = lambda shp: pl.BlockSpec(shp, lambda i: (0,) * len(shp))
    return pl.pallas_call(
        kernel,
        out_shape=jax.ShapeDtypeStruct((B, T // 4, U, D), x.dtype),
        grid=(3 * NTILE + 1,),
        in_specs=[pl.BlockSpec(memory_space=pl.ANY)] * 3 + [full((B, U, D)), full((D, D)), full((D, D)), full((D, D))],
        out_specs=pl.BlockSpec(memory_space=pl.ANY),
        scratch_shapes=[
            pltpu.VMEM((8192, 256), BF16),
            pltpu.VMEM((2, XPAD * R, 128), U32),
            pltpu.VMEM((31, 256, 256), BF16),
            pltpu.VMEM((31, 256, 256), BF16),
            pltpu.VMEM((2, 81, 256, 256), U32),
            pltpu.VMEM((3, 16, 2, 128, 128), U32),
            pltpu.VMEM((3, 27, 64, 512), U32),
            pltpu.VMEM((3, 27, 2, 128, 128), F32),
            pltpu.VMEM((3, 3, 15, 2, 144, 128), F32),
            pltpu.VMEM((16, 64, 256), U32),
            pltpu.VMEM((16, 128, 256), F32),
            pltpu.VMEM((2, 8, 256), F32),
            pltpu.VMEM((128, 256), U32),
            pltpu.VMEM((128, 256), U32),
            pltpu.VMEM((NCH, CH * 16, 8, 256), BF16),
            pltpu.SemaphoreType.DMA((1,)),
            pltpu.SemaphoreType.DMA((2,)),
            pltpu.SemaphoreType.DMA((NCH,)),
        ],
        compiler_params=pltpu.CompilerParams(
            dimension_semantics=("arbitrary",),
            vmem_limit_bytes=127 * 1024 * 1024,
        ),
    )(x, w1, w2, g, w_f, w_g, w_o)
```

```python
import functools, math
import jax
import jax.numpy as jnp
import numpy as np
from jax import lax
from jax.experimental import pallas as pl
from jax.experimental.pallas import tpu as pltpu

F32, BF16, U32 = jnp.float32, jnp.bfloat16, jnp.uint32
R = 128
JT = 125
XPAD = 33
GP = 8
NCH = 5
CH = JT // NCH
PC = 5
NTILE = 4
HI_MASK = np.uint32(0xFFFF0000)


def _bc(x, ty):
    return pltpu.bitcast(x, ty)


def _pack(a, b):
    return pltpu.pack_elementwise([a, b], packed_dtype=BF16)


def _lo(w):
    return _bc(w << 16, F32)


def _hi(w):
    return _bc(w & HI_MASK, F32)


def _expand(a):
    if len(a) == 1:
        return [a[0]]
    m = len(a) // 2
    lo, hi = a[:m], a[m:]
    return _expand(lo) + _expand(hi) + _expand([p - q for p, q in zip(lo, hi)])


def _comb(p0, p1, p2, m):
    n = 2 * m - 1
    mid = [p0[k] + p1[k] - p2[k] for k in range(n)]
    out = []
    for k in range(4 * m - 1):
        terms = []
        if k < n:
            terms.append(p0[k])
        if 0 <= k - m < n:
            terms.append(mid[k - m])
        if 0 <= k - 2 * m < n:
            terms.append(p1[k - 2 * m])
        s = terms[0]
        for t in terms[1:]:
            s = s + t
        out.append(s)
    return out


def _interp(p):
    if len(p) == 1:
        return [p[0]]
    n3 = len(p) // 3
    L = round(math.log(len(p), 3))
    ch = [_interp(p[i * n3:(i + 1) * n3]) for i in range(3)]
    return _comb(ch[0], ch[1], ch[2], 2 ** (L - 1))


def _expand_pairs(a, b, emit, base=0):
    if len(a) == 1:
        emit(base, a[0], b[0])
        return
    m = len(a) // 2
    n3 = 3 ** (m.bit_length() - 1)
    _expand_pairs(a[:m], b[:m], emit, base)
    _expand_pairs(a[m:], b[m:], emit, base + n3)
    _expand_pairs([p - q for p, q in zip(a[:m], a[m:])], [p - q for p, q in zip(b[:m], b[m:])], emit, base + 2 * n3)


def _interp_lazy(load, base, L):
    if L == 0:
        return [load(base)]
    n3 = 3 ** (L - 1)
    ch = [_interp_lazy(load, base + i * n3, L - 1) for i in range(3)]
    return _comb(ch[0], ch[1], ch[2], 2 ** (L - 1))


def _gelu_half(u):
    c = 0.7978845608028654
    inner = u * (2.0 * c + (8.0 * c * 0.044715) * (u * u))
    return u + u * jnp.tanh(inner)


def _interleave(backbone, fillers):
    nb, nf = len(backbone), len(fillers)
    done = 0
    for i, bb in enumerate(backbone):
        bb()
        upto = ((i + 1) * nf) // nb
        while done < upto:
            fillers[done]()
            done += 1
    while done < nf:
        fillers[done]()
        done += 1


def kernel(x_hbm, w1_hbm, w2_hbm, g_hbm, wf_hbm, wg_hbm, wo_hbm, o_hbm,
           xbuf, xs, wst1, wst2, wts, raws, lsc, psc, gsc, fsc, fesc, gesc, wfs, wos, ost, g_ref, wsm,
           xsem, wsem, osem, ssem):
    k = pl.program_id(0)
    tile = k // 3
    ph = k % 3

    def x_copy(t, hf):
        bb = t // 2
        if hf == 0:
            return pltpu.make_async_copy(x_hbm.at[bb, pl.ds(0, 8128)], xbuf.at[pl.ds(64, 8128)], xsem.at[0])
        return pltpu.make_async_copy(x_hbm.at[bb, pl.ds(7936, 8064)], xbuf.at[pl.ds(0, 8064)], xsem.at[0])

    def x_start(t):
        def act(hf):
            x_copy(t, hf).start()
            lo, n = (0, 64) if hf == 0 else (8064, 128)
            xbuf[pl.ds(lo, n), :] = jnp.zeros((n, 256), BF16)
        if isinstance(t, int):
            act(t % 2)
        else:
            pl.when(t % 2 == 0)(functools.partial(act, 0))
            pl.when(t % 2 == 1)(functools.partial(act, 1))

    def x_wait(t):
        def act(hf):
            x_copy(t, hf).wait()
        if isinstance(t, int):
            act(t % 2)
        else:
            pl.when(t % 2 == 0)(functools.partial(act, 0))
            pl.when(t % 2 == 1)(functools.partial(act, 1))

    def o_piece(t, c, p):
        return pltpu.make_async_copy(
            ost.at[c, pl.ds(p * PC * 16, PC * 16)],
            o_hbm.at[t // 2, pl.ds((t % 2) * 2000 + (c * CH + p * PC) * 16, PC * 16)], osem.at[c])

    def o_wait(c):
        pltpu.make_async_copy(ost.at[c], ost.at[c], osem.at[c]).wait()

    def transform_w(wst, cv):
        def body(i, carry):
            r0 = pl.multiple_of(i * 16, 16)
            for e in range(2):
                for ct in range(2):
                    lo, hi = [], []
                    for j in range(16):
                        idx = 29 - 2 * j + e
                        if idx < 0:
                            lo.append(jnp.zeros((8, 128), F32))
                            hi.append(jnp.zeros((8, 128), F32))
                        else:
                            w = _bc(wst[idx, pl.ds(r0, 16), pl.ds(128 * ct, 128)], U32)
                            lo.append(_lo(w) * 0.5)
                            hi.append(_hi(w) * 0.5)
                    la, lb = _expand(lo), _expand(hi)
                    for q in range(81):
                        wts[cv, q, pl.ds(pl.multiple_of(128 * e + i * 8, 8), 8), pl.ds(128 * ct, 128)] = _pack(la[q], lb[q])
            return carry
        lax.fori_loop(0, 16, body, 0)

    def transform_item(wst, cv, i, e, ct):
        def f():
            lo, hi = [], []
            for j in range(16):
                idx = 29 - 2 * j + e
                if idx < 0:
                    lo.append(jnp.zeros((8, 128), F32))
                    hi.append(jnp.zeros((8, 128), F32))
                else:
                    w = _bc(wst[idx, pl.ds(16 * i, 16), pl.ds(128 * ct, 128)], U32)
                    lo.append(_lo(w) * 0.5)
                    hi.append(_hi(w) * 0.5)

            def emit(q, a, b):
                wts[cv, q, pl.ds(128 * e + 8 * i, 8), pl.ds(128 * ct, 128)] = _pack(a, b)
            _expand_pairs(lo, hi, emit)
        return f

    def xcopy_item(rho, ct):
        def f():
            slot = 32 * (rho % 4) + rho // 4
            xs[ct, pl.ds(XPAD * slot, 32), :] = _bc(xbuf[pl.ds(64 * rho, 64), pl.ds(128 * ct, 128)], U32)
        return f

    def xcopy_items():
        return [xcopy_item(rho, ct) for rho in range(R) for ct in range(2)]

    def rawprep_item(c, r, ct, qs=tuple(range(8))):
        def f():
            for q in qs:
                for ab in range(2):
                    cls = (q // 4) + 2 * ab
                    raws[c, r, ct, pl.ds(64 * ab + 8 * q, 8), :] = xs[
                        ct, pl.ds(XPAD * (32 * cls + 8 * (q % 4)) + 16 * c + r, 8, stride=XPAD), :]
        return f

    def rawprep_items():
        return [rawprep_item(c, r, ct) for c in range(2) for r in range(16) for ct in range(2)]

    def pre_item(rs, g, q, kap):
        def f():
            e, ct = divmod(kap, 2)
            un = _lo if e == 0 else _hi

            def load(r, ab):
                return un(raws[rs, r, ct, pl.ds(64 * ab + 8 * q, 8), :])
            ops = []
            for ab in range(2):
                if g == 0:
                    ops.append([load(r, ab) for r in range(8)])
                elif g == 1:
                    ops.append([load(r + 8, ab) for r in range(8)])
                else:
                    ops.append([load(r, ab) - load(r + 8, ab) for r in range(8)])

            def emit(l, a, b):
                lsc[g, l, pl.ds(8 * q, 8), pl.ds(128 * kap, 128)] = _pack(a, b)
            _expand_pairs(ops[0], ops[1], emit)
        return f

    def pre_items(rs, g):
        return [pre_item(rs, g, q, kap) for q in range(8) for kap in range(4)]

    def mm_item(cv, g, l):
        def f():
            if (g, l) == (1, 13):
                lhs = _bc(lsc[g, l, :, pl.ds(256, 256)], BF16)
                rhs = _bc(wts[cv, 27 * g + l, pl.ds(128, 128), :], BF16)
            else:
                lhs = _bc(lsc[g, l], BF16)
                rhs = _bc(wts[cv, 27 * g + l], BF16)
            res = jnp.dot(lhs, rhs, preferred_element_type=F32)
            for ct in range(2):
                psc[g, l, ct] = res[:, 128 * ct:128 * (ct + 1)]
        return f

    def mm_items(cv, g):
        return [mm_item(cv, g, l) for l in range(27)]

    def post_item(gslot, g, chunk, ct):
        def f():
            row0 = 8 * chunk
            co = _interp_lazy(lambda l: psc[g, l, ct, pl.ds(row0, 8), :], 0, 3)
            for kk in range(15):
                gsc[gslot, g, kk, ct, pl.ds(GP + row0, 8), :] = co[kk]
        return f

    def post_items(gslot, g):
        return [post_item(gslot, g, chunk, ct) for chunk in range(16) for ct in range(2)]

    def G(gslot, g, kk, ct, row, n):
        return gsc[gslot, g, kk, ct, pl.ds(GP + row, n), :]

    def own(gslot, r, ct, row, n):
        def M(kk):
            return G(gslot, 0, kk, ct, row, n) + G(gslot, 1, kk, ct, row, n) - G(gslot, 2, kk, ct, row, n)
        if r == 0:
            return G(gslot, 0, 7, ct, row, n)
        if r <= 7:
            return G(gslot, 0, r + 7, ct, row, n) + M(r - 1)
        if r == 8:
            return M(7)
        return G(gslot, 1, r - 9, ct, row, n) + M(r - 1)

    def final1_item(t, q, eo, ct):
        def f():
            half = t % 2
            row = 64 * eo + 8 * q
            need_mask = eo == 0 and q in (0, 7)
            if need_mask:
                rows = lax.broadcasted_iota(jnp.int32, (8, 128), 0)
                bad = jnp.where(half == 0, 0, 8) if q == 0 else jnp.where(half == 0, 8, 7)
                keep = rows != bad
            prev_row = (64 + 8 * q - 1) if eo == 0 else 8 * q
            next_row = (64 + 8 * q) if eo == 0 else 8 * q + 1
            for c in range(2):
                hs = []
                for r in range(16):
                    y = own(c, r, ct, row, 8)
                    if r <= 7:
                        y = y + (G(1, 1, r + 7, ct, prev_row, 8) if c == 0 else G(0, 1, r + 7, ct, row, 8))
                    if r >= 9:
                        y = y + (G(1, 0, r - 9, ct, row, 8) if c == 0 else G(0, 0, r - 9, ct, next_row, 8))
                    h = _gelu_half(y)
                    if need_mask:
                        h = jnp.where(keep, h, 0.0)
                    hs.append(h)
                for rp in range(8):
                    raws[2, 8 * c + rp, ct, pl.ds(row, 8), :] = _pack(hs[2 * rp], hs[2 * rp + 1])
        return f

    def final1_items(t):
        return [final1_item(t, q, eo, ct) for q in range(8) for eo in range(2) for ct in range(2)]

    def final2_item(chunk, ct):
        def f():
            row0 = 16 * chunk
            for r in range(16):
                y = own(2, r, ct, row0, 16)
                if r <= 7:
                    y = y + G(2, 1, r + 7, ct, row0 - 1, 16)
                if r >= 9:
                    y = y + G(2, 0, r - 9, ct, row0 + 1, 16)
                fv = _gelu_half(y)
                fsc[r, pl.ds(8 * chunk, 8), pl.ds(128 * ct, 128)] = _pack(fv[0:8], fv[8:16])
        return f

    def final2_items():
        return [final2_item(chunk, ct) for chunk in range(8) for ct in range(2)]

    def fe_item(r):
        def f():
            fe = jnp.dot(_bc(fsc[r], BF16), _bc(wfs[...], BF16), preferred_element_type=F32)
            for ct in range(2):
                fesc[r, ct] = fe[:, 128 * ct:128 * (ct + 1)]
        return f

    def fe_items():
        return [fe_item(r) for r in range(16)]

    def joint_item(t, i):
        def f():
            rho = i + 1
            m = 16 * (rho // 16) + (2 * (rho % 16) if rho % 16 < 8 else 2 * (rho % 16 - 8) + 1)
            ge = [gesc[t // 2, ct] for ct in range(2)]
            rows = [jnp.concatenate([jnp.tanh(fesc[r, ct, pl.ds(m, 8, stride=0), :] + ge[ct]) for ct in range(2)], axis=1)
                    for r in range(16)]
            j = jnp.concatenate(rows, axis=0).astype(BF16)
            res = jnp.dot(j, _bc(wos[...], BF16), preferred_element_type=F32)
            c, ii = divmod(i, CH)
            ost[c, pl.ds(16 * ii, 16)] = res.reshape(16, 8, 256).astype(BF16)
            if (ii + 1) % PC == 0:
                o_piece(t, c, ii // PC).start()
        return f

    def joint_items(t):
        return [joint_item(t, i) for i in range(JT)]

    def gap_items(t):
        return (post_items(1, 2) + final1_items(t) + xcopy_items() + rawprep_items() + pre_items(2, 0))

    def unit_body():
        cv = jnp.where(ph == 2, 1, 0)
        nxt = (ph + 1) % 3
        prv = (ph + 2) % 3
        _interleave(mm_items(cv, 0), post_items(prv, 2) + pre_items(ph, 1))
        _interleave(mm_items(cv, 1), post_items(ph, 0) + pre_items(ph, 2))
        _interleave(mm_items(cv, 2), post_items(ph, 1) + pre_items(nxt, 0))

    def w_copy(i):
        return pltpu.make_async_copy((w1_hbm, w2_hbm)[i], (wst1, wst2)[i], wsem.at[i])

    def x0_copy(i):
        lo = max(2048 * i, 64)
        n = 2048 * (i + 1) - lo
        return pltpu.make_async_copy(x_hbm.at[0, pl.ds(lo - 64, n)], xbuf.at[pl.ds(lo, n)], xsem.at[i])

    def small_copy(i):
        src = (wf_hbm, wg_hbm, wo_hbm, g_hbm)[i]
        dst = g_ref if i == 3 else wsm.at[i]
        return pltpu.make_async_copy(src, dst, ssem.at[i])

    @pl.when(k == 0)
    def _():
        w_copy(0).start()
        for i in range(4):
            small_copy(i).start()
        xbuf[pl.ds(0, 64), :] = jnp.zeros((64, 256), BF16)
        for kk in range(15):
            for gg in range(2):
                gsc[2, gg, kk] = jnp.zeros((2, R + 2 * GP, 128), F32)
        for l in range(27):
            psc[2, l] = jnp.zeros((2, R, 128), F32)
        w_copy(0).wait()
        for i in range(4):
            x0_copy(i).start()
        transform_w(wst1, 0)
        for i in range(4):
            small_copy(i).wait()
        wfs[...] = _bc(wsm[0], U32)
        wos[...] = _bc(wsm[2], U32)
        for bb in range(2):
            gev = jnp.dot(g_ref[bb], wsm[1], preferred_element_type=F32)
            for ct in range(2):
                gesc[bb, ct] = gev[:, 128 * ct:128 * (ct + 1)]
        xc, pr = xcopy_items(), pre_items(0, 0)
        for i in range(4):
            x0_copy(i).wait()
            for it in xc[64 * i:64 * (i + 1)]:
                it()
            for c in range(2):
                for r in range(16):
                    for ct in range(2):
                        rawprep_item(c, r, ct, (i, i + 4))()
            for q in (i, i + 4):
                for it in pr[4 * q:4 * q + 4]:
                    it()
        w_copy(1).start()

    @pl.when(jnp.logical_and(ph == 0, tile + 1 < NTILE))
    def _():
        x_start(tile + 1)

    mid = jnp.logical_or(ph == 2, k == 3 * NTILE)

    @pl.when(jnp.logical_and(ph == 2, tile + 1 < NTILE))
    def _():
        x_wait(tile + 1)

    @pl.when(jnp.logical_and(mid, k > 5))
    def _():
        for c in range(NCH):
            o_wait(c)

    @pl.when(k == 2)
    def _():
        w_copy(1).wait()
        for it in gap_items(tile) + [transform_item(wst2, 1, i, e, ct) for i in range(16) for e in range(2) for ct in range(2)]:
            it()

    @pl.when(k == 3 * NTILE)
    def _():
        with jax.named_scope('tail'):
            for it in post_items(2, 2):
                it()

    @pl.when(jnp.logical_and(mid, k > 2))
    def _():
        jt = jnp.where(k == 3 * NTILE, NTILE - 1, tile - 1)
        ji = joint_items(jt)
        f1 = final1_items(tile)
        pr = pre_items(2, 0)
        def fq(a, b):
            return [it for q in range(a, b) for it in f1[4 * q:4 * q + 4] + pr[4 * q:4 * q + 4]]
        xc = xcopy_items()
        rp = rawprep_items()
        with jax.named_scope('B1_head'):
            for it in final2_items() + post_items(1, 2) + fe_items():
                it()
        parts = [xc + fq(0, 1), fq(1, 3), fq(3, 5), fq(5, 7), fq(7, 8) + rp]
        for c in range(NCH):
            with jax.named_scope('B1_%d' % c):
                _interleave(ji[c * CH:(c + 1) * CH], parts[c])

    @pl.when(k < 3 * NTILE)
    def _():
        with jax.named_scope('unit'):
            unit_body()

    @pl.when(k == 3 * NTILE)
    def _():
        for c in range(NCH):
            o_wait(c)


@jax.jit
def pallas_standalone__seq2seq_rnn_t_joint__speech_kernel(x, w1, w2, g, w_f, w_g, w_o):
    B, T, D = x.shape
    U = g.shape[1]
    assert (B, T, D, U) == (2, 16000, 256, 8) and w1.shape == (31, 256, 256)
    return pl.pallas_call(
        kernel,
        out_shape=jax.ShapeDtypeStruct((B, T // 4, U, D), x.dtype),
        grid=(3 * NTILE + 1,),
        in_specs=[pl.BlockSpec(memory_space=pl.ANY)] * 7,
        out_specs=pl.BlockSpec(memory_space=pl.ANY),
        scratch_shapes=[
            pltpu.VMEM((8192, 256), BF16),
            pltpu.VMEM((2, XPAD * R, 128), U32),
            pltpu.VMEM((31, 256, 256), BF16),
            pltpu.VMEM((31, 256, 256), BF16),
            pltpu.VMEM((2, 81, 256, 256), U32),
            pltpu.VMEM((3, 16, 2, 128, 128), U32),
            pltpu.VMEM((3, 27, 64, 512), U32),
            pltpu.VMEM((3, 27, 2, 128, 128), F32),
            pltpu.VMEM((3, 3, 15, 2, 144, 128), F32),
            pltpu.VMEM((16, 64, 256), U32),
            pltpu.VMEM((16, 2, 128, 128), F32),
            pltpu.VMEM((2, 2, 8, 128), F32),
            pltpu.VMEM((128, 256), U32),
            pltpu.VMEM((128, 256), U32),
            pltpu.VMEM((NCH, CH * 16, 8, 256), BF16),
            pltpu.VMEM((B, U, D), BF16),
            pltpu.VMEM((3, D, D), BF16),
            pltpu.SemaphoreType.DMA((4,)),
            pltpu.SemaphoreType.DMA((2,)),
            pltpu.SemaphoreType.DMA((NCH,)),
            pltpu.SemaphoreType.DMA((4,)),
        ],
        compiler_params=pltpu.CompilerParams(
            dimension_semantics=("arbitrary",),
            vmem_limit_bytes=127 * 1024 * 1024,
        ),
    )(x, w1, w2, g, w_f, w_g, w_o)
```

```python
import functools, math
import jax
import jax.numpy as jnp
import numpy as np
from jax import lax
from jax.experimental import pallas as pl
from jax.experimental.pallas import tpu as pltpu

F32, BF16, U32 = jnp.float32, jnp.bfloat16, jnp.uint32
R = 128
JT = 125
XPAD = 33
GP = 8
NCH = 5
CH = JT // NCH
PC = 5
NTILE = 4
HI_MASK = np.uint32(0xFFFF0000)


def _bc(x, ty):
    return pltpu.bitcast(x, ty)


def _pack(a, b):
    return pltpu.pack_elementwise([a, b], packed_dtype=BF16)


def _lo(w):
    return _bc(w << 16, F32)


def _hi(w):
    return _bc(w & HI_MASK, F32)


def _expand(a):
    if len(a) == 1:
        return [a[0]]
    m = len(a) // 2
    lo, hi = a[:m], a[m:]
    return _expand(lo) + _expand(hi) + _expand([p - q for p, q in zip(lo, hi)])


def _comb(p0, p1, p2, m):
    n = 2 * m - 1
    mid = [p0[k] + p1[k] - p2[k] for k in range(n)]
    out = []
    for k in range(4 * m - 1):
        terms = []
        if k < n:
            terms.append(p0[k])
        if 0 <= k - m < n:
            terms.append(mid[k - m])
        if 0 <= k - 2 * m < n:
            terms.append(p1[k - 2 * m])
        s = terms[0]
        for t in terms[1:]:
            s = s + t
        out.append(s)
    return out


def _interp(p):
    if len(p) == 1:
        return [p[0]]
    n3 = len(p) // 3
    L = round(math.log(len(p), 3))
    ch = [_interp(p[i * n3:(i + 1) * n3]) for i in range(3)]
    return _comb(ch[0], ch[1], ch[2], 2 ** (L - 1))


def _expand_pairs(a, b, emit, base=0):
    if len(a) == 1:
        emit(base, a[0], b[0])
        return
    m = len(a) // 2
    n3 = 3 ** (m.bit_length() - 1)
    _expand_pairs(a[:m], b[:m], emit, base)
    _expand_pairs(a[m:], b[m:], emit, base + n3)
    _expand_pairs([p - q for p, q in zip(a[:m], a[m:])], [p - q for p, q in zip(b[:m], b[m:])], emit, base + 2 * n3)


def _interp_lazy(load, base, L):
    if L == 0:
        return [load(base)]
    n3 = 3 ** (L - 1)
    ch = [_interp_lazy(load, base + i * n3, L - 1) for i in range(3)]
    return _comb(ch[0], ch[1], ch[2], 2 ** (L - 1))


def _gelu_half(u):
    c = 0.7978845608028654
    inner = u * (2.0 * c + (8.0 * c * 0.044715) * (u * u))
    return u + u * jnp.tanh(inner)


def _interleave(backbone, fillers):
    nb, nf = len(backbone), len(fillers)
    done = 0
    for i, bb in enumerate(backbone):
        bb()
        upto = ((i + 1) * nf) // nb
        while done < upto:
            fillers[done]()
            done += 1
    while done < nf:
        fillers[done]()
        done += 1


def kernel(x_hbm, w1_hbm, w2_hbm, g_hbm, wf_hbm, wg_hbm, wo_hbm, o_hbm,
           xbuf, xs, wst1, wst2, wts, raws, lsc, psc, gsc, fsc, fesc, gesc, wfs, wos, ost, g_ref, wsm,
           xsem, wsem, osem, ssem):
    k = pl.program_id(0)
    tile = k // 3
    ph = k % 3

    def x_copy(t, hf):
        bb = t // 2
        if hf == 0:
            return pltpu.make_async_copy(x_hbm.at[bb, pl.ds(0, 8128)], xbuf.at[pl.ds(64, 8128)], xsem.at[0])
        return pltpu.make_async_copy(x_hbm.at[bb, pl.ds(7936, 8064)], xbuf.at[pl.ds(0, 8064)], xsem.at[0])

    def x_start(t):
        def act(hf):
            x_copy(t, hf).start()
            lo, n = (0, 64) if hf == 0 else (8064, 128)
            xbuf[pl.ds(lo, n), :] = jnp.zeros((n, 256), BF16)
        if isinstance(t, int):
            act(t % 2)
        else:
            pl.when(t % 2 == 0)(functools.partial(act, 0))
            pl.when(t % 2 == 1)(functools.partial(act, 1))

    def x_wait(t):
        def act(hf):
            x_copy(t, hf).wait()
        if isinstance(t, int):
            act(t % 2)
        else:
            pl.when(t % 2 == 0)(functools.partial(act, 0))
            pl.when(t % 2 == 1)(functools.partial(act, 1))

    def o_piece(t, c, p):
        return pltpu.make_async_copy(
            ost.at[c, pl.ds(p * PC * 16, PC * 16)],
            o_hbm.at[t // 2, pl.ds((t % 2) * 2000 + (c * CH + p * PC) * 16, PC * 16)], osem.at[c])

    def o_wait(c):
        pltpu.make_async_copy(ost.at[c], ost.at[c], osem.at[c]).wait()

    def transform_w(wst, cv):
        def body(i, carry):
            r0 = pl.multiple_of(i * 16, 16)
            for e in range(2):
                for ct in range(2):
                    lo, hi = [], []
                    for j in range(16):
                        idx = 29 - 2 * j + e
                        if idx < 0:
                            lo.append(jnp.zeros((8, 128), F32))
                            hi.append(jnp.zeros((8, 128), F32))
                        else:
                            w = _bc(wst[idx, pl.ds(r0, 16), pl.ds(128 * ct, 128)], U32)
                            lo.append(_lo(w) * 0.5)
                            hi.append(_hi(w) * 0.5)
                    la, lb = _expand(lo), _expand(hi)
                    for q in range(81):
                        wts[cv, q, pl.ds(pl.multiple_of(128 * e + i * 8, 8), 8), pl.ds(128 * ct, 128)] = _pack(la[q], lb[q])
            return carry
        lax.fori_loop(0, 16, body, 0)

    def transform_item(wst, cv, i, e, ct):
        def f():
            lo, hi = [], []
            for j in range(16):
                idx = 29 - 2 * j + e
                if idx < 0:
                    lo.append(jnp.zeros((8, 128), F32))
                    hi.append(jnp.zeros((8, 128), F32))
                else:
                    w = _bc(wst[idx, pl.ds(16 * i, 16), pl.ds(128 * ct, 128)], U32)
                    lo.append(_lo(w) * 0.5)
                    hi.append(_hi(w) * 0.5)

            def emit(q, a, b):
                wts[cv, q, pl.ds(128 * e + 8 * i, 8), pl.ds(128 * ct, 128)] = _pack(a, b)
            _expand_pairs(lo, hi, emit)
        return f

    def xcopy_item(rho, ct):
        def f():
            slot = 32 * (rho % 4) + rho // 4
            xs[ct, pl.ds(XPAD * slot, 32), :] = _bc(xbuf[pl.ds(64 * rho, 64), pl.ds(128 * ct, 128)], U32)
        return f

    def xcopy_items():
        return [xcopy_item(rho, ct) for rho in range(R) for ct in range(2)]

    def rawprep_item(c, r, ct, qs=tuple(range(8))):
        def f():
            for q in qs:
                for ab in range(2):
                    cls = (q // 4) + 2 * ab
                    raws[c, r, ct, pl.ds(64 * ab + 8 * q, 8), :] = xs[
                        ct, pl.ds(XPAD * (32 * cls + 8 * (q % 4)) + 16 * c + r, 8, stride=XPAD), :]
        return f

    def rawprep_items():
        return [rawprep_item(c, r, ct) for c in range(2) for r in range(16) for ct in range(2)]

    def pre_item(rs, g, q, kap):
        def f():
            e, ct = divmod(kap, 2)
            un = _lo if e == 0 else _hi

            def load(r, ab):
                return un(raws[rs, r, ct, pl.ds(64 * ab + 8 * q, 8), :])
            ops = []
            for ab in range(2):
                if g == 0:
                    ops.append([load(r, ab) for r in range(8)])
                elif g == 1:
                    ops.append([load(r + 8, ab) for r in range(8)])
                else:
                    ops.append([load(r, ab) - load(r + 8, ab) for r in range(8)])

            def emit(l, a, b):
                lsc[g, l, pl.ds(8 * q, 8), pl.ds(128 * kap, 128)] = _pack(a, b)
            _expand_pairs(ops[0], ops[1], emit)
        return f

    def pre_items(rs, g):
        return [pre_item(rs, g, q, kap) for q in range(8) for kap in range(4)]

    def mm_item(cv, g, l):
        def f():
            if (g, l) == (1, 13):
                lhs = _bc(lsc[g, l, :, pl.ds(256, 256)], BF16)
                rhs = _bc(wts[cv, 27 * g + l, pl.ds(128, 128), :], BF16)
            else:
                lhs = _bc(lsc[g, l], BF16)
                rhs = _bc(wts[cv, 27 * g + l], BF16)
            res = jnp.dot(lhs, rhs, preferred_element_type=F32)
            for ct in range(2):
                psc[g, l, ct] = res[:, 128 * ct:128 * (ct + 1)]
        return f

    def mm_items(cv, g):
        return [mm_item(cv, g, l) for l in range(27)]

    def post_item(gslot, g, chunk, ct):
        def f():
            row0 = 8 * chunk
            co = _interp_lazy(lambda l: psc[g, l, ct, pl.ds(row0, 8), :], 0, 3)
            if g < 2:
                for kk in range(15):
                    gsc[gslot, g, kk, ct, pl.ds(GP + row0, 8), :] = co[kk]
                return
            g0 = [gsc[gslot, 0, kk, ct, pl.ds(GP + row0, 8), :] for kk in range(15)]
            g1 = [gsc[gslot, 1, kk, ct, pl.ds(GP + row0, 8), :] for kk in range(15)]
            for r in range(1, 16):
                mid = g0[r - 1] + g1[r - 1] - co[r - 1]
                if r <= 7:
                    mid = mid + g0[r + 7]
                elif r >= 9:
                    mid = mid + g1[r - 9]
                gsc[gslot, 2, r - 1, ct, pl.ds(GP + row0, 8), :] = mid
        return f

    def post_items(gslot, g):
        return [post_item(gslot, g, chunk, ct) for chunk in range(16) for ct in range(2)]

    def G(gslot, g, kk, ct, row, n):
        return gsc[gslot, g, kk, ct, pl.ds(GP + row, n), :]

    def own(gslot, r, ct, row, n):
        if r == 0:
            return G(gslot, 0, 7, ct, row, n)
        return G(gslot, 2, r - 1, ct, row, n)

    def final1_item(t, q, eo, ct):
        def f():
            half = t % 2
            row = 64 * eo + 8 * q
            need_mask = eo == 0 and q in (0, 7)
            if need_mask:
                rows = lax.broadcasted_iota(jnp.int32, (8, 128), 0)
                bad = jnp.where(half == 0, 0, 8) if q == 0 else jnp.where(half == 0, 8, 7)
                keep = rows != bad
            prev_row = (64 + 8 * q - 1) if eo == 0 else 8 * q
            next_row = (64 + 8 * q) if eo == 0 else 8 * q + 1
            for c in range(2):
                hs = []
                for r in range(16):
                    y = own(c, r, ct, row, 8)
                    if r <= 7:
                        y = y + (G(1, 1, r + 7, ct, prev_row, 8) if c == 0 else G(0, 1, r + 7, ct, row, 8))
                    if r >= 9:
                        y = y + (G(1, 0, r - 9, ct, row, 8) if c == 0 else G(0, 0, r - 9, ct, next_row, 8))
                    h = _gelu_half(y)
                    if need_mask:
                        h = jnp.where(keep, h, 0.0)
                    hs.append(h)
                for rp in range(8):
                    raws[2, 8 * c + rp, ct, pl.ds(row, 8), :] = _pack(hs[2 * rp], hs[2 * rp + 1])
        return f

    def final1_items(t):
        return [final1_item(t, q, eo, ct) for q in range(8) for eo in range(2) for ct in range(2)]

    def final2_item(chunk, ct):
        def f():
            row0 = 16 * chunk
            for r in range(16):
                y = own(2, r, ct, row0, 16)
                if r <= 7:
                    y = y + G(2, 1, r + 7, ct, row0 - 1, 16)
                if r >= 9:
                    y = y + G(2, 0, r - 9, ct, row0 + 1, 16)
                fv = _gelu_half(y)
                fsc[r, pl.ds(8 * chunk, 8), pl.ds(128 * ct, 128)] = _pack(fv[0:8], fv[8:16])
        return f

    def final2_items():
        return [final2_item(chunk, ct) for chunk in range(8) for ct in range(2)]

    def fe_item(r):
        def f():
            fe = jnp.dot(_bc(fsc[r], BF16), _bc(wfs[...], BF16), preferred_element_type=F32)
            for ct in range(2):
                fesc[r, ct] = fe[:, 128 * ct:128 * (ct + 1)]
        return f

    def fe_items():
        return [fe_item(r) for r in range(16)]

    def joint_item(t, i):
        def f():
            rho = i + 1
            m = 16 * (rho // 16) + (2 * (rho % 16) if rho % 16 < 8 else 2 * (rho % 16 - 8) + 1)
            ge = [gesc[t // 2, ct] for ct in range(2)]
            rows = [jnp.concatenate([jnp.tanh(fesc[r, ct, pl.ds(m, 8, stride=0), :] + ge[ct]) for ct in range(2)], axis=1)
                    for r in range(16)]
            j = jnp.concatenate(rows, axis=0).astype(BF16)
            res = jnp.dot(j, _bc(wos[...], BF16), preferred_element_type=F32)
            c, ii = divmod(i, CH)
            ost[c, pl.ds(16 * ii, 16)] = res.reshape(16, 8, 256).astype(BF16)
            if (ii + 1) % PC == 0:
                o_piece(t, c, ii // PC).start()
        return f

    def joint_items(t):
        return [joint_item(t, i) for i in range(JT)]

    def gap_items(t):
        return final1_items(t) + xcopy_items() + rawprep_items() + pre_items(2, 0)

    def unit_body():
        cv = jnp.where(ph == 2, 1, 0)
        nxt = (ph + 1) % 3
        _interleave(mm_items(cv, 0), pre_items(ph, 1))
        _interleave(mm_items(cv, 1), post_items(ph, 0) + pre_items(ph, 2))
        _interleave(mm_items(cv, 2), post_items(ph, 1) + pre_items(nxt, 0))
        for it in post_items(ph, 2):
            it()

    def w_copy(i):
        return pltpu.make_async_copy((w1_hbm, w2_hbm)[i], (wst1, wst2)[i], wsem.at[i])

    def x0_copy(i):
        lo = max(2048 * i, 64)
        n = 2048 * (i + 1) - lo
        return pltpu.make_async_copy(x_hbm.at[0, pl.ds(lo - 64, n)], xbuf.at[pl.ds(lo, n)], xsem.at[i])

    def small_copy(i):
        src = (wf_hbm, wg_hbm, wo_hbm, g_hbm)[i]
        dst = g_ref if i == 3 else wsm.at[i]
        return pltpu.make_async_copy(src, dst, ssem.at[i])

    @pl.when(k == 0)
    def _():
        w_copy(0).start()
        for i in range(4):
            small_copy(i).start()
        xbuf[pl.ds(0, 64), :] = jnp.zeros((64, 256), BF16)
        for kk in range(15):
            for gg in range(2):
                gsc[2, gg, kk] = jnp.zeros((2, R + 2 * GP, 128), F32)
        w_copy(0).wait()
        for i in range(4):
            x0_copy(i).start()
        transform_w(wst1, 0)
        for i in range(4):
            small_copy(i).wait()
        wfs[...] = _bc(wsm[0], U32)
        wos[...] = _bc(wsm[2], U32)
        for bb in range(2):
            gev = jnp.dot(g_ref[bb], wsm[1], preferred_element_type=F32)
            for ct in range(2):
                gesc[bb, ct] = gev[:, 128 * ct:128 * (ct + 1)]
        xc, pr = xcopy_items(), pre_items(0, 0)
        for i in range(4):
            x0_copy(i).wait()
            for it in xc[64 * i:64 * (i + 1)]:
                it()
            for c in range(2):
                for r in range(16):
                    for ct in range(2):
                        rawprep_item(c, r, ct, (i, i + 4))()
            for q in (i, i + 4):
                for it in pr[4 * q:4 * q + 4]:
                    it()
        w_copy(1).start()

    @pl.when(jnp.logical_and(ph == 0, tile + 1 < NTILE))
    def _():
        x_start(tile + 1)

    mid = jnp.logical_or(ph == 2, k == 3 * NTILE)

    @pl.when(jnp.logical_and(ph == 2, tile + 1 < NTILE))
    def _():
        x_wait(tile + 1)

    @pl.when(jnp.logical_and(mid, k > 5))
    def _():
        for c in range(NCH):
            o_wait(c)

    @pl.when(k == 2)
    def _():
        w_copy(1).wait()
        for it in gap_items(tile) + [transform_item(wst2, 1, i, e, ct) for i in range(16) for e in range(2) for ct in range(2)]:
            it()

    @pl.when(jnp.logical_and(mid, k > 2))
    def _():
        jt = jnp.where(k == 3 * NTILE, NTILE - 1, tile - 1)
        ji = joint_items(jt)
        f1 = final1_items(tile)
        pr = pre_items(2, 0)
        def fq(a, b):
            return [it for q in range(a, b) for it in f1[4 * q:4 * q + 4] + pr[4 * q:4 * q + 4]]
        xc = xcopy_items()
        rp = rawprep_items()
        with jax.named_scope('B1_head'):
            for it in final2_items() + fe_items():
                it()
        parts = [xc + fq(0, 1), fq(1, 3), fq(3, 5), fq(5, 7), fq(7, 8) + rp]
        for c in range(NCH):
            with jax.named_scope('B1_%d' % c):
                _interleave(ji[c * CH:(c + 1) * CH], parts[c])

    @pl.when(k < 3 * NTILE)
    def _():
        with jax.named_scope('unit'):
            unit_body()

    @pl.when(k == 3 * NTILE)
    def _():
        for c in range(NCH):
            o_wait(c)


@jax.jit
def pallas_standalone__seq2seq_rnn_t_joint__speech_kernel(x, w1, w2, g, w_f, w_g, w_o):
    B, T, D = x.shape
    U = g.shape[1]
    assert (B, T, D, U) == (2, 16000, 256, 8) and w1.shape == (31, 256, 256)
    return pl.pallas_call(
        kernel,
        out_shape=jax.ShapeDtypeStruct((B, T // 4, U, D), x.dtype),
        grid=(3 * NTILE + 1,),
        in_specs=[pl.BlockSpec(memory_space=pl.ANY)] * 7,
        out_specs=pl.BlockSpec(memory_space=pl.ANY),
        scratch_shapes=[
            pltpu.VMEM((8192, 256), BF16),
            pltpu.VMEM((2, XPAD * R, 128), U32),
            pltpu.VMEM((31, 256, 256), BF16),
            pltpu.VMEM((31, 256, 256), BF16),
            pltpu.VMEM((2, 81, 256, 256), U32),
            pltpu.VMEM((3, 16, 2, 128, 128), U32),
            pltpu.VMEM((3, 27, 64, 512), U32),
            pltpu.VMEM((3, 27, 2, 128, 128), F32),
            pltpu.VMEM((3, 3, 15, 2, 144, 128), F32),
            pltpu.VMEM((16, 64, 256), U32),
            pltpu.VMEM((16, 2, 128, 128), F32),
            pltpu.VMEM((2, 2, 8, 128), F32),
            pltpu.VMEM((128, 256), U32),
            pltpu.VMEM((128, 256), U32),
            pltpu.VMEM((NCH, CH * 16, 8, 256), BF16),
            pltpu.VMEM((B, U, D), BF16),
            pltpu.VMEM((3, D, D), BF16),
            pltpu.SemaphoreType.DMA((4,)),
            pltpu.SemaphoreType.DMA((2,)),
            pltpu.SemaphoreType.DMA((NCH,)),
            pltpu.SemaphoreType.DMA((4,)),
        ],
        compiler_params=pltpu.CompilerParams(
            dimension_semantics=("arbitrary",),
            vmem_limit_bytes=127 * 1024 * 1024,
        ),
    )(x, w1, w2, g, w_f, w_g, w_o)
```

```python
import functools
import jax
import jax.numpy as jnp
import numpy as np
from jax import lax
from jax.experimental import pallas as pl
from jax.experimental.pallas import tpu as pltpu

F32, BF16, U32 = jnp.float32, jnp.bfloat16, jnp.uint32
R = 128
JT = 125
XPAD = 33
GP = 8
NCH = 5
CH = JT // NCH
PC = 5
NTILE = 4
HI_MASK = np.uint32(0xFFFF0000)


def _bc(x, ty):
    return pltpu.bitcast(x, ty)


def _pack(a, b):
    return pltpu.pack_elementwise([a, b], packed_dtype=BF16)


def _lo(w):
    return _bc(w << 16, F32)


def _hi(w):
    return _bc(w & HI_MASK, F32)


def _expand(a):
    if len(a) == 1:
        return [a[0]]
    m = len(a) // 2
    lo, hi = a[:m], a[m:]
    return _expand(lo) + _expand(hi) + _expand([p - q for p, q in zip(lo, hi)])


def _comb(p0, p1, p2, m):
    n = 2 * m - 1
    mid = [p0[k] + p1[k] - p2[k] for k in range(n)]
    out = []
    for k in range(4 * m - 1):
        terms = []
        if k < n:
            terms.append(p0[k])
        if 0 <= k - m < n:
            terms.append(mid[k - m])
        if 0 <= k - 2 * m < n:
            terms.append(p1[k - 2 * m])
        s = terms[0]
        for t in terms[1:]:
            s = s + t
        out.append(s)
    return out


def _expand_pairs(a, b, emit, base=0):
    if len(a) == 1:
        emit(base, a[0], b[0])
        return
    m = len(a) // 2
    n3 = 3 ** (m.bit_length() - 1)
    _expand_pairs(a[:m], b[:m], emit, base)
    _expand_pairs(a[m:], b[m:], emit, base + n3)
    _expand_pairs([p - q for p, q in zip(a[:m], a[m:])], [p - q for p, q in zip(b[:m], b[m:])], emit, base + 2 * n3)


def _interp_lazy(load, base, L):
    if L == 0:
        return [load(base)]
    n3 = 3 ** (L - 1)
    ch = [_interp_lazy(load, base + i * n3, L - 1) for i in range(3)]
    return _comb(ch[0], ch[1], ch[2], 2 ** (L - 1))


def _gelu_half(u):
    c = 0.7978845608028654
    inner = u * (2.0 * c + (8.0 * c * 0.044715) * (u * u))
    return u + u * jnp.tanh(inner)


def _interleave(backbone, fillers):
    nb, nf = len(backbone), len(fillers)
    done = 0
    for i, bb in enumerate(backbone):
        bb()
        upto = ((i + 1) * nf) // nb
        while done < upto:
            fillers[done]()
            done += 1
    while done < nf:
        fillers[done]()
        done += 1


def kernel(x_hbm, w1_hbm, w2_hbm, g_hbm, wf_hbm, wg_hbm, wo_hbm, o_hbm,
           xbuf, xs, wst1, wst2, wts, raws, lsc, psc, gsc, fsc, fesc, gesc, wfs, wos, ost, g_ref, wsm,
           xsem, wsem, osem, ssem):
    k = pl.program_id(0)
    tile = k // 3
    ph = k % 3

    def x_copy(t, hf):
        bb = t // 2
        if hf == 0:
            return pltpu.make_async_copy(x_hbm.at[bb, pl.ds(0, 8128)], xbuf.at[pl.ds(64, 8128)], xsem.at[0])
        return pltpu.make_async_copy(x_hbm.at[bb, pl.ds(7936, 8064)], xbuf.at[pl.ds(0, 8064)], xsem.at[0])

    def x_start(t):
        def act(hf):
            x_copy(t, hf).start()
            lo, n = (0, 64) if hf == 0 else (8064, 128)
            xbuf[pl.ds(lo, n), :] = jnp.zeros((n, 256), BF16)
        if isinstance(t, int):
            act(t % 2)
        else:
            pl.when(t % 2 == 0)(functools.partial(act, 0))
            pl.when(t % 2 == 1)(functools.partial(act, 1))

    def x_wait(t):
        def act(hf):
            x_copy(t, hf).wait()
        if isinstance(t, int):
            act(t % 2)
        else:
            pl.when(t % 2 == 0)(functools.partial(act, 0))
            pl.when(t % 2 == 1)(functools.partial(act, 1))

    def o_piece(t, c, p):
        return pltpu.make_async_copy(
            ost.at[c, pl.ds(p * PC * 16, PC * 16)],
            o_hbm.at[t // 2, pl.ds((t % 2) * 2000 + (c * CH + p * PC) * 16, PC * 16)], osem.at[c])

    def o_wait(c):
        pltpu.make_async_copy(ost.at[c], ost.at[c], osem.at[c]).wait()

    def transform_w(wst, cv):
        def body(i, carry):
            r0 = pl.multiple_of(i * 16, 16)
            for e in range(2):
                for ct in range(2):
                    lo, hi = [], []
                    for j in range(16):
                        idx = 29 - 2 * j + e
                        if idx < 0:
                            lo.append(jnp.zeros((8, 128), F32))
                            hi.append(jnp.zeros((8, 128), F32))
                        else:
                            w = _bc(wst[idx, pl.ds(r0, 16), pl.ds(128 * ct, 128)], U32)
                            lo.append(_lo(w) * 0.5)
                            hi.append(_hi(w) * 0.5)
                    la, lb = _expand(lo), _expand(hi)
                    for q in range(81):
                        wts[cv, q, pl.ds(pl.multiple_of(128 * e + i * 8, 8), 8), pl.ds(128 * ct, 128)] = _pack(la[q], lb[q])
            return carry
        lax.fori_loop(0, 16, body, 0)

    def transform_item(wst, cv, i, e, ct):
        def f():
            lo, hi = [], []
            for j in range(16):
                idx = 29 - 2 * j + e
                if idx < 0:
                    lo.append(jnp.zeros((8, 128), F32))
                    hi.append(jnp.zeros((8, 128), F32))
                else:
                    w = _bc(wst[idx, pl.ds(16 * i, 16), pl.ds(128 * ct, 128)], U32)
                    lo.append(_lo(w) * 0.5)
                    hi.append(_hi(w) * 0.5)

            def emit(q, a, b):
                wts[cv, q, pl.ds(128 * e + 8 * i, 8), pl.ds(128 * ct, 128)] = _pack(a, b)
            _expand_pairs(lo, hi, emit)
        return f

    def xcopy_item(rho, ct):
        def f():
            slot = 32 * (rho % 4) + rho // 4
            xs[ct, pl.ds(XPAD * slot, 32), :] = _bc(xbuf[pl.ds(64 * rho, 64), pl.ds(128 * ct, 128)], U32)
        return f

    def xcopy_items():
        return [xcopy_item(rho, ct) for rho in range(R) for ct in range(2)]

    def rawprep_item(c, r, ct, qs=tuple(range(8))):
        def f():
            for q in qs:
                for ab in range(2):
                    cls = (q // 4) + 2 * ab
                    raws[c, r, ct, pl.ds(64 * ab + 8 * q, 8), :] = xs[
                        ct, pl.ds(XPAD * (32 * cls + 8 * (q % 4)) + 16 * c + r, 8, stride=XPAD), :]
        return f

    def rawprep_items():
        return [rawprep_item(c, r, ct) for c in range(2) for r in range(16) for ct in range(2)]

    def pre_item(rs, g, q, kap):
        def f():
            e, ct = divmod(kap, 2)
            un = _lo if e == 0 else _hi

            def load(r, ab):
                return un(raws[rs, r, ct, pl.ds(64 * ab + 8 * q, 8), :])
            ops = []
            for ab in range(2):
                if g == 0:
                    ops.append([load(r, ab) for r in range(8)])
                elif g == 1:
                    ops.append([load(r + 8, ab) for r in range(8)])
                else:
                    ops.append([load(r, ab) - load(r + 8, ab) for r in range(8)])

            def emit(l, a, b):
                lsc[g, l, pl.ds(8 * q, 8), pl.ds(128 * kap, 128)] = _pack(a, b)
            _expand_pairs(ops[0], ops[1], emit)
        return f

    def pre_items(rs, g):
        return [pre_item(rs, g, q, kap) for q in range(8) for kap in range(4)]

    def mm_item(cv, g, l):
        def f():
            if (g, l) == (1, 13):
                lhs = _bc(lsc[g, l, :, pl.ds(256, 256)], BF16)
                rhs = _bc(wts[cv, 27 * g + l, pl.ds(128, 128), :], BF16)
            else:
                lhs = _bc(lsc[g, l], BF16)
                rhs = _bc(wts[cv, 27 * g + l], BF16)
            res = jnp.dot(lhs, rhs, preferred_element_type=F32)
            for ct in range(2):
                psc[g, l, ct] = res[:, 128 * ct:128 * (ct + 1)]
        return f

    def mm_items(cv, g):
        return [mm_item(cv, g, l) for l in range(27)]

    def post_item(gslot, g, chunk, ct):
        def f():
            row0 = 8 * chunk
            co = _interp_lazy(lambda l: psc[g, l, ct, pl.ds(row0, 8), :], 0, 3)
            if g < 2:
                for kk in range(15):
                    gsc[gslot, g, kk, ct, pl.ds(GP + row0, 8), :] = co[kk]
                return
            g0 = [gsc[gslot, 0, kk, ct, pl.ds(GP + row0, 8), :] for kk in range(15)]
            g1 = [gsc[gslot, 1, kk, ct, pl.ds(GP + row0, 8), :] for kk in range(15)]
            for r in range(1, 16):
                mid = g0[r - 1] + g1[r - 1] - co[r - 1]
                if r <= 7:
                    mid = mid + g0[r + 7]
                elif r >= 9:
                    mid = mid + g1[r - 9]
                gsc[gslot, 2, r - 1, ct, pl.ds(GP + row0, 8), :] = mid
        return f

    def post_items(gslot, g):
        return [post_item(gslot, g, chunk, ct) for chunk in range(16) for ct in range(2)]

    def G(gslot, g, kk, ct, row, n):
        return gsc[gslot, g, kk, ct, pl.ds(GP + row, n), :]

    def own(gslot, r, ct, row, n):
        if r == 0:
            return G(gslot, 0, 7, ct, row, n)
        return G(gslot, 2, r - 1, ct, row, n)

    def final1_item(t, q, eo, ct):
        def f():
            half = t % 2
            row = 64 * eo + 8 * q
            need_mask = eo == 0 and q in (0, 7)
            if need_mask:
                rows = lax.broadcasted_iota(jnp.int32, (8, 128), 0)
                bad = jnp.where(half == 0, 0, 8) if q == 0 else jnp.where(half == 0, 8, 7)
                keep = rows != bad
            prev_row = (64 + 8 * q - 1) if eo == 0 else 8 * q
            next_row = (64 + 8 * q) if eo == 0 else 8 * q + 1
            for c in range(2):
                hs = []
                for r in range(16):
                    y = own(c, r, ct, row, 8)
                    if r <= 7:
                        y = y + (G(1, 1, r + 7, ct, prev_row, 8) if c == 0 else G(0, 1, r + 7, ct, row, 8))
                    if r >= 9:
                        y = y + (G(1, 0, r - 9, ct, row, 8) if c == 0 else G(0, 0, r - 9, ct, next_row, 8))
                    h = _gelu_half(y)
                    if need_mask:
                        h = jnp.where(keep, h, 0.0)
                    hs.append(h)
                for rp in range(8):
                    raws[2, 8 * c + rp, ct, pl.ds(row, 8), :] = _pack(hs[2 * rp], hs[2 * rp + 1])
        return f

    def final1_items(t):
        return [final1_item(t, q, eo, ct) for q in range(8) for eo in range(2) for ct in range(2)]

    def final2_item(chunk, ct):
        def f():
            row0 = 16 * chunk
            for r in range(16):
                y = own(2, r, ct, row0, 16)
                if r <= 7:
                    y = y + G(2, 1, r + 7, ct, row0 - 1, 16)
                if r >= 9:
                    y = y + G(2, 0, r - 9, ct, row0 + 1, 16)
                fv = _gelu_half(y)
                fsc[r, pl.ds(8 * chunk, 8), pl.ds(128 * ct, 128)] = _pack(fv[0:8], fv[8:16])
        return f

    def final2_items():
        return [final2_item(chunk, ct) for chunk in range(8) for ct in range(2)]

    def fe_item(r):
        def f():
            fe = jnp.dot(_bc(fsc[r], BF16), _bc(wfs[...], BF16), preferred_element_type=F32)
            for ct in range(2):
                fesc[r, ct] = fe[:, 128 * ct:128 * (ct + 1)]
        return f

    def fe_items():
        return [fe_item(r) for r in range(16)]

    def joint_item(t, i):
        def f():
            rho = i + 1
            m = 16 * (rho // 16) + (2 * (rho % 16) if rho % 16 < 8 else 2 * (rho % 16 - 8) + 1)
            ge = [gesc[t // 2, ct] for ct in range(2)]
            rows = [jnp.concatenate([jnp.tanh(fesc[r, ct, pl.ds(m, 1), :] + ge[ct]) for ct in range(2)], axis=1)
                    for r in range(16)]
            j = jnp.concatenate(rows, axis=0).astype(BF16)
            res = jnp.dot(j, _bc(wos[...], BF16), preferred_element_type=F32)
            c, ii = divmod(i, CH)
            ost[c, pl.ds(16 * ii, 16)] = res.reshape(16, 8, 256).astype(BF16)
            if (ii + 1) % PC == 0:
                o_piece(t, c, ii // PC).start()
        return f

    def joint_items(t):
        return [joint_item(t, i) for i in range(JT)]

    def gap_items(t):
        return final1_items(t) + xcopy_items() + rawprep_items() + pre_items(2, 0)

    def unit_body():
        cv = jnp.where(ph == 2, 1, 0)
        nxt = (ph + 1) % 3
        _interleave(mm_items(cv, 0), pre_items(ph, 1))
        _interleave(mm_items(cv, 1), post_items(ph, 0) + pre_items(ph, 2))
        _interleave(mm_items(cv, 2), post_items(ph, 1) + pre_items(nxt, 0))
        for it in post_items(ph, 2):
            it()

    def w_copy(i):
        return pltpu.make_async_copy((w1_hbm, w2_hbm)[i], (wst1, wst2)[i], wsem.at[i])

    def x0_copy(i):
        lo = max(2048 * i, 64)
        n = 2048 * (i + 1) - lo
        return pltpu.make_async_copy(x_hbm.at[0, pl.ds(lo - 64, n)], xbuf.at[pl.ds(lo, n)], xsem.at[i])

    def small_copy(i):
        src = (wf_hbm, wg_hbm, wo_hbm, g_hbm)[i]
        dst = g_ref if i == 3 else wsm.at[i]
        return pltpu.make_async_copy(src, dst, ssem.at[i])

    @pl.when(k == 0)
    def _():
        w_copy(0).start()
        for i in range(4):
            small_copy(i).start()
        xbuf[pl.ds(0, 64), :] = jnp.zeros((64, 256), BF16)
        raws[2] = jnp.zeros((16, 2, R, 128), U32)
        for kk in range(15):
            for gg in range(2):
                gsc[2, gg, kk] = jnp.zeros((2, R + 2 * GP, 128), F32)
        w_copy(0).wait()
        for i in range(4):
            x0_copy(i).start()
        transform_w(wst1, 0)
        for i in range(4):
            small_copy(i).wait()
        wfs[...] = _bc(wsm[0], U32)
        wos[...] = _bc(wsm[2], U32)
        for bb in range(2):
            gev = jnp.dot(g_ref[bb], wsm[1], preferred_element_type=F32)
            for ct in range(2):
                gesc[bb, ct] = gev[:, 128 * ct:128 * (ct + 1)]
        xc, pr = xcopy_items(), pre_items(0, 0)
        for i in range(4):
            x0_copy(i).wait()
            for it in xc[64 * i:64 * (i + 1)]:
                it()
            for c in range(2):
                for r in range(16):
                    for ct in range(2):
                        rawprep_item(c, r, ct, (i, i + 4))()
            for q in (i, i + 4):
                for it in pr[4 * q:4 * q + 4]:
                    it()
        w_copy(1).start()

    @pl.when(jnp.logical_and(ph == 0, tile + 1 < NTILE))
    def _():
        x_start(tile + 1)

    mid = jnp.logical_or(ph == 2, k == 3 * NTILE)

    @pl.when(jnp.logical_and(ph == 2, tile + 1 < NTILE))
    def _():
        x_wait(tile + 1)

    @pl.when(jnp.logical_and(mid, k > 5))
    def _():
        for c in range(NCH):
            o_wait(c)

    @pl.when(k == 2)
    def _():
        w_copy(1).wait()
        for it in gap_items(tile) + [transform_item(wst2, 1, i, e, ct) for i in range(16) for e in range(2) for ct in range(2)]:
            it()

    @pl.when(jnp.logical_and(mid, k > 2))
    def _():
        jt = jnp.where(k == 3 * NTILE, NTILE - 1, tile - 1)
        ji = joint_items(jt)
        f1 = final1_items(tile)
        pr = pre_items(2, 0)
        def fq(a, b):
            return [it for q in range(a, b) for it in f1[4 * q:4 * q + 4] + pr[4 * q:4 * q + 4]]
        xc = xcopy_items()
        rp = rawprep_items()
        for it in final2_items() + fe_items():
            it()
        parts = [xc + fq(0, 1), fq(1, 3), fq(3, 5), fq(5, 7), fq(7, 8) + rp]
        for c in range(NCH):
            _interleave(ji[c * CH:(c + 1) * CH], parts[c])

    @pl.when(k < 3 * NTILE)
    def _():
        unit_body()

    @pl.when(k == 3 * NTILE)
    def _():
        for c in range(NCH):
            o_wait(c)


@jax.jit
def pallas_standalone__seq2seq_rnn_t_joint__speech_kernel(x, w1, w2, g, w_f, w_g, w_o):
    B, T, D = x.shape
    U = g.shape[1]
    assert (B, T, D, U) == (2, 16000, 256, 8) and w1.shape == (31, 256, 256)
    return pl.pallas_call(
        kernel,
        out_shape=jax.ShapeDtypeStruct((B, T // 4, U, D), x.dtype),
        grid=(3 * NTILE + 1,),
        in_specs=[pl.BlockSpec(memory_space=pl.ANY)] * 7,
        out_specs=pl.BlockSpec(memory_space=pl.ANY),
        scratch_shapes=[
            pltpu.VMEM((8192, 256), BF16),
            pltpu.VMEM((2, XPAD * R, 128), U32),
            pltpu.VMEM((31, 256, 256), BF16),
            pltpu.VMEM((31, 256, 256), BF16),
            pltpu.VMEM((2, 81, 256, 256), U32),
            pltpu.VMEM((3, 16, 2, 128, 128), U32),
            pltpu.VMEM((3, 27, 64, 512), U32),
            pltpu.VMEM((3, 27, 2, 128, 128), F32),
            pltpu.VMEM((3, 3, 15, 2, 144, 128), F32),
            pltpu.VMEM((16, 64, 256), U32),
            pltpu.VMEM((16, 2, 128, 128), F32),
            pltpu.VMEM((2, 2, 8, 128), F32),
            pltpu.VMEM((128, 256), U32),
            pltpu.VMEM((128, 256), U32),
            pltpu.VMEM((NCH, CH * 16, 8, 256), BF16),
            pltpu.VMEM((B, U, D), BF16),
            pltpu.VMEM((3, D, D), BF16),
            pltpu.SemaphoreType.DMA((4,)),
            pltpu.SemaphoreType.DMA((2,)),
            pltpu.SemaphoreType.DMA((NCH,)),
            pltpu.SemaphoreType.DMA((4,)),
        ],
        compiler_params=pltpu.CompilerParams(
            dimension_semantics=("arbitrary",),
            vmem_limit_bytes=127 * 1024 * 1024,
        ),
    )(x, w1, w2, g, w_f, w_g, w_o)
```

```python
import functools
import jax
import jax.numpy as jnp
import numpy as np
from jax import lax
from jax.experimental import pallas as pl
from jax.experimental.pallas import tpu as pltpu

F32, BF16, U32 = jnp.float32, jnp.bfloat16, jnp.uint32
R = 128
JT = 125
XPAD = 33
GP = 8
NCH = 5
CH = JT // NCH
PC = 5
NTILE = 4
HOFF = XPAD * R
HI_MASK = np.uint32(0xFFFF0000)


def _bc(x, ty):
    return pltpu.bitcast(x, ty)


def _pack(a, b):
    return pltpu.pack_elementwise([a, b], packed_dtype=BF16)


def _lo(w):
    return _bc(w << 16, F32)


def _hi(w):
    return _bc(w & HI_MASK, F32)


def _expand(a):
    if len(a) == 1:
        return [a[0]]
    m = len(a) // 2
    lo, hi = a[:m], a[m:]
    return _expand(lo) + _expand(hi) + _expand([p - q for p, q in zip(lo, hi)])


def _comb(p0, p1, p2, m):
    n = 2 * m - 1
    mid = [p0[k] + p1[k] - p2[k] for k in range(n)]
    out = []
    for k in range(4 * m - 1):
        terms = []
        if k < n:
            terms.append(p0[k])
        if 0 <= k - m < n:
            terms.append(mid[k - m])
        if 0 <= k - 2 * m < n:
            terms.append(p1[k - 2 * m])
        s = terms[0]
        for t in terms[1:]:
            s = s + t
        out.append(s)
    return out


def _expand_pairs(a, b, emit, base=0):
    if len(a) == 1:
        emit(base, a[0], b[0])
        return
    m = len(a) // 2
    n3 = 3 ** (m.bit_length() - 1)
    _expand_pairs(a[:m], b[:m], emit, base)
    _expand_pairs(a[m:], b[m:], emit, base + n3)
    _expand_pairs([p - q for p, q in zip(a[:m], a[m:])], [p - q for p, q in zip(b[:m], b[m:])], emit, base + 2 * n3)


def _interp_lazy(load, base, L):
    if L == 0:
        return [load(base)]
    n3 = 3 ** (L - 1)
    ch = [_interp_lazy(load, base + i * n3, L - 1) for i in range(3)]
    return _comb(ch[0], ch[1], ch[2], 2 ** (L - 1))


def _gelu_half(u):
    c = 0.7978845608028654
    inner = u * (2.0 * c + (8.0 * c * 0.044715) * (u * u))
    return u + u * jnp.tanh(inner)


def _interleave(backbone, fillers):
    nb, nf = len(backbone), len(fillers)
    done = 0
    for i, bb in enumerate(backbone):
        bb()
        upto = ((i + 1) * nf) // nb
        while done < upto:
            fillers[done]()
            done += 1
    while done < nf:
        fillers[done]()
        done += 1


def kernel(x_hbm, w1_hbm, w2_hbm, g_hbm, wf_hbm, wg_hbm, wo_hbm, o_hbm,
           xbuf, xs, wst1, wst2, wts, lsc, psc, gsc, fsc, fesc, gesc, wfs, wos, ost, g_ref, wsm,
           xsem, wsem, osem, ssem):
    k = pl.program_id(0)
    tile = k // 3
    ph = k % 3

    def x_copy(t, hf):
        bb = t // 2
        if hf == 0:
            return pltpu.make_async_copy(x_hbm.at[bb, pl.ds(0, 8128)], xbuf.at[pl.ds(64, 8128)], xsem.at[0])
        return pltpu.make_async_copy(x_hbm.at[bb, pl.ds(7936, 8064)], xbuf.at[pl.ds(0, 8064)], xsem.at[0])

    def x_start(t):
        def act(hf):
            x_copy(t, hf).start()
            lo, n = (0, 64) if hf == 0 else (8064, 128)
            xbuf[pl.ds(lo, n), :] = jnp.zeros((n, 256), BF16)
        if isinstance(t, int):
            act(t % 2)
        else:
            pl.when(t % 2 == 0)(functools.partial(act, 0))
            pl.when(t % 2 == 1)(functools.partial(act, 1))

    def x_wait(t):
        def act(hf):
            x_copy(t, hf).wait()
        if isinstance(t, int):
            act(t % 2)
        else:
            pl.when(t % 2 == 0)(functools.partial(act, 0))
            pl.when(t % 2 == 1)(functools.partial(act, 1))

    def o_piece(t, c, p):
        return pltpu.make_async_copy(
            ost.at[c, pl.ds(p * PC * 16, PC * 16)],
            o_hbm.at[t // 2, pl.ds((t % 2) * 2000 + (c * CH + p * PC) * 16, PC * 16)], osem.at[c])

    def o_wait(c):
        pltpu.make_async_copy(ost.at[c], ost.at[c], osem.at[c]).wait()

    def transform_w(wst, cv):
        def body(i, carry):
            r0 = pl.multiple_of(i * 16, 16)
            for e in range(2):
                for ct in range(2):
                    lo, hi = [], []
                    for j in range(16):
                        idx = 29 - 2 * j + e
                        if idx < 0:
                            lo.append(jnp.zeros((8, 128), F32))
                            hi.append(jnp.zeros((8, 128), F32))
                        else:
                            w = _bc(wst[idx, pl.ds(r0, 16), pl.ds(128 * ct, 128)], U32)
                            lo.append(_lo(w) * 0.5)
                            hi.append(_hi(w) * 0.5)
                    la, lb = _expand(lo), _expand(hi)
                    for q in range(81):
                        wts[cv, q, pl.ds(pl.multiple_of(128 * e + i * 8, 8), 8), pl.ds(128 * ct, 128)] = _pack(la[q], lb[q])
            return carry
        lax.fori_loop(0, 16, body, 0)

    def transform_item(wst, cv, i, e, ct):
        def f():
            lo, hi = [], []
            for j in range(16):
                idx = 29 - 2 * j + e
                if idx < 0:
                    lo.append(jnp.zeros((8, 128), F32))
                    hi.append(jnp.zeros((8, 128), F32))
                else:
                    w = _bc(wst[idx, pl.ds(16 * i, 16), pl.ds(128 * ct, 128)], U32)
                    lo.append(_lo(w) * 0.5)
                    hi.append(_hi(w) * 0.5)

            def emit(q, a, b):
                wts[cv, q, pl.ds(128 * e + 8 * i, 8), pl.ds(128 * ct, 128)] = _pack(a, b)
            _expand_pairs(lo, hi, emit)
        return f

    def xcopy_item(rho, ct):
        def f():
            slot = 32 * (rho % 4) + rho // 4
            xs[ct, pl.ds(XPAD * slot, 32), :] = _bc(xbuf[pl.ds(64 * rho, 64), pl.ds(128 * ct, 128)], U32)
        return f

    def xcopy_items():
        return [xcopy_item(rho, ct) for rho in range(R) for ct in range(2)]

    def slot_row(q, ab):
        return XPAD * (32 * ((q // 4) + 2 * ab) + 8 * (q % 4))

    def pre_item(rs, g, q, kap):
        def f():
            e, ct = divmod(kap, 2)
            un = _lo if e == 0 else _hi

            def load(r, ab):
                return un(xs[ct, pl.ds(rs + slot_row(q, ab) + r, 8, stride=XPAD), :])
            ops = []
            for ab in range(2):
                if g == 0:
                    ops.append([load(r, ab) for r in range(8)])
                elif g == 1:
                    ops.append([load(r + 8, ab) for r in range(8)])
                else:
                    ops.append([load(r, ab) - load(r + 8, ab) for r in range(8)])

            def emit(l, a, b):
                lsc[g, l, pl.ds(8 * q, 8), pl.ds(128 * kap, 128)] = _pack(a, b)
            _expand_pairs(ops[0], ops[1], emit)
        return f

    def pre_items(rs, g):
        return [pre_item(rs, g, q, kap) for q in range(8) for kap in range(4)]

    def mm_item(cv, g, l):
        def f():
            if (g, l) == (1, 13):
                lhs = _bc(lsc[g, l, :, pl.ds(256, 256)], BF16)
                rhs = _bc(wts[cv, 27 * g + l, pl.ds(128, 128), :], BF16)
            else:
                lhs = _bc(lsc[g, l], BF16)
                rhs = _bc(wts[cv, 27 * g + l], BF16)
            res = jnp.dot(lhs, rhs, preferred_element_type=F32)
            for ct in range(2):
                psc[g, l, ct] = res[:, 128 * ct:128 * (ct + 1)]
        return f

    def mm_items(cv, g):
        return [mm_item(cv, g, l) for l in range(27)]

    def post_item(gslot, g, chunk, ct):
        def f():
            row0 = 8 * chunk
            co = _interp_lazy(lambda l: psc[g, l, ct, pl.ds(row0, 8), :], 0, 3)
            if g < 2:
                for kk in range(15):
                    gsc[gslot, g, kk, ct, pl.ds(GP + row0, 8), :] = co[kk]
                return
            g0 = [gsc[gslot, 0, kk, ct, pl.ds(GP + row0, 8), :] for kk in range(15)]
            g1 = [gsc[gslot, 1, kk, ct, pl.ds(GP + row0, 8), :] for kk in range(15)]
            for r in range(1, 16):
                mid = g0[r - 1] + g1[r - 1] - co[r - 1]
                if r <= 7:
                    mid = mid + g0[r + 7]
                elif r >= 9:
                    mid = mid + g1[r - 9]
                gsc[gslot, 2, r - 1, ct, pl.ds(GP + row0, 8), :] = mid
        return f

    def post_items(gslot, g):
        return [post_item(gslot, g, chunk, ct) for chunk in range(16) for ct in range(2)]

    def G(gslot, g, kk, ct, row, n):
        return gsc[gslot, g, kk, ct, pl.ds(GP + row, n), :]

    def own(gslot, r, ct, row, n):
        if r == 0:
            return G(gslot, 0, 7, ct, row, n)
        return G(gslot, 2, r - 1, ct, row, n)

    def final1_item(t, q, eo, ct):
        def f():
            half = t % 2
            row = 64 * eo + 8 * q
            need_mask = eo == 0 and q in (0, 7)
            if need_mask:
                rows = lax.broadcasted_iota(jnp.int32, (8, 128), 0)
                bad = jnp.where(half == 0, 0, 8) if q == 0 else jnp.where(half == 0, 8, 7)
                keep = rows != bad
            prev_row = (64 + 8 * q - 1) if eo == 0 else 8 * q
            next_row = (64 + 8 * q) if eo == 0 else 8 * q + 1
            for c in range(2):
                hs = []
                for r in range(16):
                    y = own(c, r, ct, row, 8)
                    if r <= 7:
                        y = y + (G(1, 1, r + 7, ct, prev_row, 8) if c == 0 else G(0, 1, r + 7, ct, row, 8))
                    if r >= 9:
                        y = y + (G(1, 0, r - 9, ct, row, 8) if c == 0 else G(0, 0, r - 9, ct, next_row, 8))
                    h = _gelu_half(y)
                    if need_mask:
                        h = jnp.where(keep, h, 0.0)
                    hs.append(h)
                for rp in range(8):
                    xs[ct, pl.ds(HOFF + slot_row(q, eo) + 8 * c + rp, 8, stride=XPAD), :] = _pack(hs[2 * rp], hs[2 * rp + 1])
        return f

    def final1_items(t):
        return [final1_item(t, q, eo, ct) for q in range(8) for eo in range(2) for ct in range(2)]

    def final2_item(chunk, ct):
        def f():
            row0 = 16 * chunk
            for r in range(16):
                y = own(2, r, ct, row0, 16)
                if r <= 7:
                    y = y + G(2, 1, r + 7, ct, row0 - 1, 16)
                if r >= 9:
                    y = y + G(2, 0, r - 9, ct, row0 + 1, 16)
                fv = _gelu_half(y)
                fsc[r, pl.ds(8 * chunk, 8), pl.ds(128 * ct, 128)] = _pack(fv[0:8], fv[8:16])
        return f

    def final2_items():
        return [final2_item(chunk, ct) for chunk in range(8) for ct in range(2)]

    def fe_item(r):
        def f():
            fe = jnp.dot(_bc(fsc[r], BF16), _bc(wfs[...], BF16), preferred_element_type=F32)
            for ct in range(2):
                fesc[r, ct] = fe[:, 128 * ct:128 * (ct + 1)]
        return f

    def fe_items():
        return [fe_item(r) for r in range(16)]

    def joint_item(t, i):
        def f():
            rho = i + 1
            m = 16 * (rho // 16) + (2 * (rho % 16) if rho % 16 < 8 else 2 * (rho % 16 - 8) + 1)
            ge = [gesc[t // 2, ct] for ct in range(2)]
            rows = [jnp.concatenate([jnp.tanh(fesc[r, ct, pl.ds(m, 1), :] + ge[ct]) for ct in range(2)], axis=1)
                    for r in range(16)]
            j = jnp.concatenate(rows, axis=0).astype(BF16)
            res = jnp.dot(j, _bc(wos[...], BF16), preferred_element_type=F32)
            c, ii = divmod(i, CH)
            ost[c, pl.ds(16 * ii, 16)] = res.reshape(16, 8, 256).astype(BF16)
            if (ii + 1) % PC == 0:
                o_piece(t, c, ii // PC).start()
        return f

    def joint_items(t):
        return [joint_item(t, i) for i in range(JT)]

    def gap_items(t):
        return final1_items(t) + xcopy_items() + pre_items(HOFF, 0)

    def unit_body():
        cv = jnp.where(ph == 2, 1, 0)
        cur_off = jnp.where(ph == 2, HOFF, 16 * ph)
        nxt_off = jnp.where(ph == 1, HOFF, jnp.where(ph == 0, 16, 0))
        _interleave(mm_items(cv, 0), pre_items(cur_off, 1))
        _interleave(mm_items(cv, 1), post_items(ph, 0) + pre_items(cur_off, 2))
        _interleave(mm_items(cv, 2), post_items(ph, 1) + pre_items(nxt_off, 0))
        for it in post_items(ph, 2):
            it()

    def w_copy(i):
        return pltpu.make_async_copy((w1_hbm, w2_hbm)[i], (wst1, wst2)[i], wsem.at[i])

    def x0_copy(i):
        lo = max(2048 * i, 64)
        n = 2048 * (i + 1) - lo
        return pltpu.make_async_copy(x_hbm.at[0, pl.ds(lo - 64, n)], xbuf.at[pl.ds(lo, n)], xsem.at[i])

    def small_copy(i):
        src = (wf_hbm, wg_hbm, wo_hbm, g_hbm)[i]
        dst = g_ref if i == 3 else wsm.at[i]
        return pltpu.make_async_copy(src, dst, ssem.at[i])

    @pl.when(k == 0)
    def _():
        w_copy(0).start()
        for i in range(4):
            small_copy(i).start()
        xbuf[pl.ds(0, 64), :] = jnp.zeros((64, 256), BF16)
        for ct in range(2):
            xs[ct, pl.ds(HOFF, HOFF), :] = jnp.zeros((HOFF, 128), U32)
        for kk in range(15):
            for gg in range(2):
                gsc[2, gg, kk] = jnp.zeros((2, R + 2 * GP, 128), F32)
        w_copy(0).wait()
        for i in range(4):
            x0_copy(i).start()
        transform_w(wst1, 0)
        for i in range(4):
            small_copy(i).wait()
        wfs[...] = _bc(wsm[0], U32)
        wos[...] = _bc(wsm[2], U32)
        for bb in range(2):
            gev = jnp.dot(g_ref[bb], wsm[1], preferred_element_type=F32)
            for ct in range(2):
                gesc[bb, ct] = gev[:, 128 * ct:128 * (ct + 1)]
        xc, pr = xcopy_items(), pre_items(0, 0)
        for i in range(4):
            x0_copy(i).wait()
            for it in xc[64 * i:64 * (i + 1)]:
                it()
            for q in (i, i + 4):
                for it in pr[4 * q:4 * q + 4]:
                    it()
        w_copy(1).start()

    @pl.when(jnp.logical_and(ph == 0, tile + 1 < NTILE))
    def _():
        x_start(tile + 1)

    mid = jnp.logical_or(ph == 2, k == 3 * NTILE)

    @pl.when(jnp.logical_and(ph == 2, tile + 1 < NTILE))
    def _():
        x_wait(tile + 1)

    @pl.when(jnp.logical_and(mid, k > 5))
    def _():
        for c in range(NCH):
            o_wait(c)

    @pl.when(k == 2)
    def _():
        w_copy(1).wait()
        for it in gap_items(tile) + [transform_item(wst2, 1, i, e, ct) for i in range(16) for e in range(2) for ct in range(2)]:
            it()

    @pl.when(jnp.logical_and(mid, k > 2))
    def _():
        jt = jnp.where(k == 3 * NTILE, NTILE - 1, tile - 1)
        ji = joint_items(jt)
        f1 = final1_items(tile)
        pr = pre_items(HOFF, 0)
        def fq(a, b):
            return [it for q in range(a, b) for it in f1[4 * q:4 * q + 4] + pr[4 * q:4 * q + 4]]
        xc = xcopy_items()
        for it in final2_items() + fe_items():
            it()
        parts = [xc + fq(0, 1), fq(1, 3), fq(3, 5), fq(5, 7), fq(7, 8)]
        for c in range(NCH):
            _interleave(ji[c * CH:(c + 1) * CH], parts[c])

    @pl.when(k < 3 * NTILE)
    def _():
        unit_body()

    @pl.when(k == 3 * NTILE)
    def _():
        for c in range(NCH):
            o_wait(c)


@jax.jit
def pallas_standalone__seq2seq_rnn_t_joint__speech_kernel(x, w1, w2, g, w_f, w_g, w_o):
    B, T, D = x.shape
    U = g.shape[1]
    assert (B, T, D, U) == (2, 16000, 256, 8) and w1.shape == (31, 256, 256)
    return pl.pallas_call(
        kernel,
        out_shape=jax.ShapeDtypeStruct((B, T // 4, U, D), x.dtype),
        grid=(3 * NTILE + 1,),
        in_specs=[pl.BlockSpec(memory_space=pl.ANY)] * 7,
        out_specs=pl.BlockSpec(memory_space=pl.ANY),
        scratch_shapes=[
            pltpu.VMEM((8192, 256), BF16),
            pltpu.VMEM((2, 2 * HOFF, 128), U32),
            pltpu.VMEM((31, 256, 256), BF16),
            pltpu.VMEM((31, 256, 256), BF16),
            pltpu.VMEM((2, 81, 256, 256), U32),
            pltpu.VMEM((3, 27, 64, 512), U32),
            pltpu.VMEM((3, 27, 2, 128, 128), F32),
            pltpu.VMEM((3, 3, 15, 2, 144, 128), F32),
            pltpu.VMEM((16, 64, 256), U32),
            pltpu.VMEM((16, 2, 128, 128), F32),
            pltpu.VMEM((2, 2, 8, 128), F32),
            pltpu.VMEM((128, 256), U32),
            pltpu.VMEM((128, 256), U32),
            pltpu.VMEM((NCH, CH * 16, 8, 256), BF16),
            pltpu.VMEM((B, U, D), BF16),
            pltpu.VMEM((3, D, D), BF16),
            pltpu.SemaphoreType.DMA((4,)),
            pltpu.SemaphoreType.DMA((2,)),
            pltpu.SemaphoreType.DMA((NCH,)),
            pltpu.SemaphoreType.DMA((4,)),
        ],
        compiler_params=pltpu.CompilerParams(
            dimension_semantics=("arbitrary",),
            vmem_limit_bytes=127 * 1024 * 1024,
        ),
    )(x, w1, w2, g, w_f, w_g, w_o)
```
